```python
import os as _os
_os.environ.setdefault("JAX_PLATFORMS", "cpu")
import jax
import jax.numpy as jnp

def _softmax(x, axis=-1):
    return jax.nn.softmax(x, axis=axis)
def _gelu(x):
    return jax.nn.gelu(x, approximate=True)
def _silu(x):
    return jax.nn.silu(x)
def _sigmoid(x):
    return jax.nn.sigmoid(x)
def _layernorm(x, axis=-1, eps=1e-5):
    m = jnp.mean(x, axis=axis, keepdims=True)
    v = jnp.var(x, axis=axis, keepdims=True)
    return (x - m) / jnp.sqrt(v + eps)
def _scatter_add(tgt, idx, src, axis=0):
    return tgt.at[idx].add(src)
def _segment_sum(src, seg, n):
    return jax.ops.segment_sum(src, seg, n)
class _Rng:
    def __init__(self, key):
        self._k = key
    def _next(self):
        self._k, sub = jax.random.split(self._k)
        return sub
    def normal(self, shape):
        return jax.random.normal(self._next(), shape, dtype=jnp.bfloat16)
    def randint(self, lo, hi, shape):
        return jax.random.randint(self._next(), shape, lo, hi, dtype=jnp.int32)
    def uniform(self, shape, lo=0.0, hi=1.0):
        return jax.random.uniform(self._next(), shape, jnp.bfloat16, lo, hi)
    def permutation(self, n):
        return jax.random.permutation(self._next(), n)


kernel_name = 'sequential_preLN__spectral_gfnet__glu_gated_bilinear__prompt'

def setup_inputs():
    _rng = _Rng(jax.random.key(int.from_bytes(__import__("os").urandom(4), "little")))
    _w = (lambda a: (lambda t: t.astype(jnp.bfloat16) if jnp.issubdtype(t.dtype, jnp.floating) else t)(jnp.asarray(a)))
    def _A_setup():
        B, S, D = 1, 2048, 448
        Df = D // 2 + 1
        return {
            "x": _w((lambda *s: _rng.normal(s) * 0.05)(B, S, D)),
            "w_r": _w((lambda *s: _rng.normal(s) * 0.2)(S, Df) * 0.02),
            "w_i": _w((lambda *s: _rng.normal(s) * 0.2)(S, Df) * 0.02),
        }
    _A_in = _A_setup()

    def _B_setup():
        B, S, D, F = 1, 2048, 448, 1792
        return {
            "x": _w((lambda *s: _rng.normal(s) * 0.05)(B, S, D)),
            "w_gate": _w((lambda *s: _rng.normal(s) * 0.05)(D, F) * (D ** -0.5)),
            "w_up": _w((lambda *s: _rng.normal(s) * 0.05)(D, F) * (D ** -0.5)),
            "w_down": _w((lambda *s: _rng.normal(s) * 0.05)(F, D) * (F ** -0.5)),
        }
    _B_in = _B_setup()

    return {
        "A_x": _A_in["x"],
        "A_w_r": _A_in["w_r"],
        "A_w_i": _A_in["w_i"],
        "B_x": _B_in["x"],
        "B_w_gate": _B_in["w_gate"],
        "B_w_up": _B_in["w_up"],
        "B_w_down": _B_in["w_down"],
    }

def reference(A_x, A_w_r, A_w_i, B_x, B_w_gate, B_w_up, B_w_down):
    def _A_ref(x, w_r, w_i):
        B, S, D = x.shape
        X = (lambda x, axes=(-2,-1): jnp.fft.rfft2(x.astype(jnp.float32), axes=axes))(x, axes=(-2, -1))
        W = w_r + 1j * w_i
        X = X * W
        y = (lambda x, s, axes=(-2,-1): jnp.fft.irfft2(x, s=s, axes=axes).astype(jnp.bfloat16))(X, (S, D), axes=(-2, -1))
        return y

    def _B_ref(x, w_gate, w_up, w_down):
        g = jnp.einsum("bsd,df->bsf", x, w_gate)
        u = jnp.einsum("bsd,df->bsf", x, w_up)
        h = g * u
        return jnp.einsum("bsf,fd->bsd", h, w_down)

    x = A_x
    h = x + _A_ref(_layernorm(x, axis=-1), A_w_r, A_w_i)
    h2 = h + _B_ref(_layernorm(h, axis=-1), B_w_gate, B_w_up, B_w_down)
    return h2
```

```python
import numpy as np
import jax
import jax.numpy as jnp
import jax.experimental.pallas as pl
import jax.experimental.pallas.tpu as pltpu

S, D, F, K = 2048, 448, 1792, 225
NT16 = 16
EPS = 1e-5
bf16, f32, u32 = jnp.bfloat16, jnp.float32, jnp.uint32
NTDIMS = (((1,), (1,)), ((), ()))
BM = 512
FC = 896


def _tables():
    import ml_dtypes
    th = 2 * np.pi / D
    n = []
    for v in range(7):
        n += [16 * v + 2 * i for i in range(8)] + [16 * v + 2 * i + 1 for i in range(8)]
    nu = np.array(n) + 0.5
    kE = 2 * np.arange(113)
    kO = 2 * np.arange(112) + 1
    Ft = np.zeros((4, 128, 128))
    Ft[0, :113, :112] = np.cos(np.outer(kE, nu) * th)
    Ft[0, 112, :] = 0
    Ft[1, :113, :112] = -np.sin(np.outer(kE, nu) * th)
    Ft[1, 0, :] = 0
    Ft[2, :112, :112] = np.cos(np.outer(kO, nu) * th)
    Ft[3, :112, :112] = -np.sin(np.outer(kO, nu) * th)
    nun = np.arange(112) + 0.5
    cE = np.full(113, 2.0)
    cE[0] = 1
    cE[112] = 1
    sc = 1.0 / (D * S)
    G = np.zeros((4, 112, 128))
    gce = np.cos(np.outer(nun, kE) * th)
    gce[:, 112] = 0
    gse = np.sin(np.outer(nun, kE) * th)
    gse[:, 0] = 0
    G[0, :, :113] = gce * cE * sc
    G[1, :, :113] = gse * cE * sc
    G[2, :, :112] = np.cos(np.outer(nun, kO) * th) * 2 * sc
    G[3, :, :112] = np.sin(np.outer(nun, kO) * th) * 2 * sc
    a = np.arange(128)
    M = np.zeros((16, 2, 128, 128))
    for d in range(16):
        ph = -2 * np.pi * ((np.outer(a, a) % 128) / 128 + (d * a / 2048)[:, None])
        M[d, 0] = np.cos(ph)
        M[d, 1] = np.sin(ph)
    b = ml_dtypes.bfloat16
    return Ft.astype(b), G.astype(b), M.astype(b)


class Sg:
    __slots__ = ("v", "s")

    def __init__(self, v, s=1):
        self.v, self.s = v, s

    def __neg__(self):
        return Sg(self.v, -self.s)

    def __add__(self, o):
        if self.s == o.s:
            return Sg(self.v + o.v, self.s)
        if self.s > 0:
            return Sg(self.v - o.v, 1)
        return Sg(o.v - self.v, 1)

    def __sub__(self, o):
        return self + (-o)

    def scale(self, c):
        return Sg(self.v * np.float32(c * self.s), 1)

    def val(self):
        return self.v if self.s > 0 else -self.v


def _dft4(x, sgn):
    (r0, i0), (r1, i1), (r2, i2), (r3, i3) = x
    t0 = (r0 + r2, i0 + i2)
    t1 = (r0 - r2, i0 - i2)
    t2 = (r1 + r3, i1 + i3)
    t3 = (r1 - r3, i1 - i3)
    X0 = (t0[0] + t2[0], t0[1] + t2[1])
    X2 = (t0[0] - t2[0], t0[1] - t2[1])
    XA = (t1[0] + t3[1], t1[1] - t3[0])
    XB = (t1[0] - t3[1], t1[1] + t3[0])
    if sgn < 0:
        return [X0, XA, X2, XB]
    return [X0, XB, X2, XA]


def _tw16(z, e, sgn):
    r, i = z
    e = e % 16
    if e == 0:
        return z
    if e == 4:
        return (i, -r) if sgn < 0 else (-i, r)
    if e == 8:
        return (-r, -i)
    h = float(np.sqrt(0.5))
    if e in (2, 6):
        c = h if e == 2 else -h
        s = h * sgn
        re = (r if c > 0 else -r) - (i if s > 0 else -i)
        im = (r if s > 0 else -r) + (i if c > 0 else -i)
        return (re.scale(h), im.scale(h))
    c = float(np.cos(2 * np.pi * e / 16))
    s = float(sgn * np.sin(2 * np.pi * e / 16))
    return (r.scale(c) - i.scale(s), r.scale(s) + i.scale(c))


def _fft16(x, sgn):
    x = [(Sg(r), Sg(i)) for r, i in x]
    U = [_dft4([x[4 * b1 + b0] for b1 in range(4)], sgn) for b0 in range(4)]
    V = [[_tw16(U[b0][d0], d0 * b0, sgn) for d0 in range(4)] for b0 in range(4)]
    out = [None] * 16
    for d0 in range(4):
        X = _dft4([V[b0][d0] for b0 in range(4)], sgn)
        for d1 in range(4):
            out[d0 + 4 * d1] = (X[d1][0].val(), X[d1][1].val())
    return out


def _unpack(u):
    lo = pltpu.bitcast(u << 16, f32)
    hi = pltpu.bitcast(u & np.uint32(0xFFFF0000), f32)
    return lo, hi


def _kernel(x_hbm, wr_hbm, wi_hbm, wg_hbm, wu_hbm, wd_hbm, f_hbm, g_hbm, m_hbm, o_hbm,
            XS, WS, WT, WP, ZS, TS, FS, GS, MS, WG, WU, WD, OS, sem_x, sem_w, sem_t, sem_m, sem_o):
    ct = [pltpu.make_async_copy(f_hbm, FS, sem_t.at[0]),
          pltpu.make_async_copy(g_hbm, GS, sem_t.at[1]),
          pltpu.make_async_copy(m_hbm, MS, sem_t.at[2])]
    cx = [pltpu.make_async_copy(x_hbm.at[:, pl.ds(t * 128, 128)], XS.at[t], sem_x.at[t]) for t in range(16)]
    cw = [[pltpu.make_async_copy(w.at[:, pl.ds(t * 128, 128)], WS.at[c, t], sem_w.at[c, t]) for t in range(16)]
          for c, w in enumerate((wr_hbm, wi_hbm))]
    cm = [pltpu.make_async_copy(a, b, sem_m.at[i])
          for i, (a, b) in enumerate(((wg_hbm, WG), (wu_hbm, WU), (wd_hbm, WD)))]
    ct[0].start()
    for c in cx:
        c.start()
    ct[2].start()
    for t in range(16):
        cw[0][t].start()
        cw[1][t].start()
    ct[1].start()
    for c in cm:
        c.start()

    row8 = jax.lax.broadcasted_iota(jnp.int32, (8, 128), 0)
    rev8 = 7 - row8

    ct[0].wait()

    def p1a(t):
        def ld(v, reverse):
            u = pltpu.bitcast(XS[t, pl.ds(16 * v, 16), :], u32)
            if reverse:
                u = jnp.take_along_axis(u, rev8, axis=0)
            return _unpack(u)
        Ree, Ro, Ie, Io = [], [], [], []
        for v in range(7):
            Al, Ah = ld(v, False)
            Bl, Bh = ld(27 - v, True)
            Cl, Ch = ld(13 - v, True)
            Dl, Dh = ld(14 + v, False)
            for (a, b, c, d) in ((Al, Bh, Ch, Dl), (Ah, Bl, Cl, Dh)):
                p = a + b
                q = c + d
                r = a - b
                s = d - c
                Ree.append(q + p)
                Ro.append(q - p)
                Ie.append(s + r)
                Io.append(s - r)
        tot = Ree[0]
        for z in Ree[1:]:
            tot = tot + z
        mean4 = jnp.sum(tot, axis=0, keepdims=True) * np.float32(4.0 / D)
        Ree = [z - mean4 for z in Ree]
        sq = None
        for lst in (Ree, Ro, Ie, Io):
            for z in lst:
                sq = z * z if sq is None else sq + z * z
        var = jnp.sum(sq, axis=0, keepdims=True) * np.float32(1.0 / (4 * D))
        rstd = jax.lax.rsqrt(var + EPS)
        zpad = jnp.zeros((16, 128), bf16)
        for blk, lst in enumerate((Ree, Ie, Ro, Io)):
            data = jnp.concatenate([jnp.concatenate(lst, axis=0).astype(bf16), zpad], axis=0)
            nrow = 128 if blk < 2 else 112
            z = jnp.dot(FS[blk, 0:nrow, :], data, preferred_element_type=f32) * rstd
            c = blk % 2
            odd = blk // 2
            for g in range(15 - odd):
                ZS[c, t, pl.ds(16 * g + 8 * odd, 8), :] = z[8 * g:8 * g + 8, :]

    for t in range(16):
        cx[t].wait()
        p1a(t)

    def s1_body(g, carry):
        r0 = pl.multiple_of(g * 8, 8)
        x = [(ZS[0, b, pl.ds(r0, 8), :], ZS[1, b, pl.ds(r0, 8), :]) for b in range(16)]
        T = _fft16(x, -1)
        q0 = pl.multiple_of(g * 16, 16)
        for d in range(16):
            TS[d, pl.ds(q0, 16), :] = jnp.concatenate([T[d][0], T[d][1]], axis=0).astype(bf16)
        return carry
    jax.lax.fori_loop(0, 29, s1_body, 0)

    def t1_body(t, carry):
        for c in range(2):
            u = pltpu.bitcast(WS[c, t, 0:224, :], u32)
            w224 = pltpu.bitcast(WS[c, t, 224:225, :].astype(f32), u32) >> 16
            last = jnp.where(row8 == 0, jnp.broadcast_to(w224, (8, 128)), np.uint32(0))
            full = jnp.concatenate([u, last, jnp.zeros((8, 128), u32)], axis=0)
            WT[c, t] = pltpu.bitcast(full, f32).T
        return carry
    for t in range(16):
        cw[0][t].wait()
        cw[1][t].wait()
    jax.lax.fori_loop(0, 16, t1_body, 0)

    def t2_body(d, carry):
        for c in range(2):
            Gm = jnp.concatenate([WT[c, t, pl.ds(d, 8, stride=16), :] for t in range(16)], axis=0)
            WP[c, d] = Gm.T[0:120, :]
        return carry
    jax.lax.fori_loop(0, 16, t2_body, 0)

    ct[2].wait()

    def s2_body(d, carry):
        lhs = TS[d]
        Mr = MS[d, 0]
        Mi = MS[d, 1]
        A = jnp.dot(lhs, Mr, preferred_element_type=f32)
        B = jnp.dot(lhs, Mi, preferred_element_type=f32)
        P = []
        for gg in range(15):
            wrl, wrh = _unpack(pltpu.bitcast(WP[0, d, pl.ds(8 * gg, 8), :], u32))
            wil, wih = _unpack(pltpu.bitcast(WP[1, d, pl.ds(8 * gg, 8), :], u32))
            for odd in range(2):
                gam = 2 * gg + odd
                if gam >= 29:
                    continue
                wr_, wi_ = (wrl, wil) if odd == 0 else (wrh, wih)
                zr = A[16 * gam:16 * gam + 8] - B[16 * gam + 8:16 * gam + 16]
                zi = B[16 * gam:16 * gam + 8] + A[16 * gam + 8:16 * gam + 16]
                P.append(zr * wr_ - zi * wi_)
                P.append(zr * wi_ + zi * wr_)
        Pb = jnp.concatenate(P, axis=0).astype(bf16)
        A2 = jax.lax.dot_general(Pb, Mr, NTDIMS, preferred_element_type=f32)
        B2 = jax.lax.dot_general(Pb, Mi, NTDIMS, preferred_element_type=f32)
        for gam in range(29):
            ZS[0, d, pl.ds(8 * gam, 8), :] = A2[16 * gam:16 * gam + 8] + B2[16 * gam + 8:16 * gam + 16]
            ZS[1, d, pl.ds(8 * gam, 8), :] = A2[16 * gam + 8:16 * gam + 16] - B2[16 * gam:16 * gam + 8]
        return carry
    jax.lax.fori_loop(0, 16, s2_body, 0)

    def s1i_body(g, carry):
        r0 = pl.multiple_of(g * 8, 8)
        x = [(ZS[0, b, pl.ds(r0, 8), :], ZS[1, b, pl.ds(r0, 8), :]) for b in range(16)]
        Y = _fft16(x, +1)
        for b in range(16):
            ZS[0, b, pl.ds(r0, 8), :] = Y[b][0]
            ZS[1, b, pl.ds(r0, 8), :] = Y[b][1]
        return carry
    jax.lax.fori_loop(0, 29, s1i_body, 0)

    ct[1].wait()
    for c in cm:
        c.wait()
    NTB = BM // 128

    def revrows(z):
        nq = z.shape[0] // 8
        idx = 7 - jax.lax.broadcasted_iota(jnp.int32, (8, z.shape[1]), 0)
        return jnp.concatenate(
            [jnp.take_along_axis(z[8 * q:8 * q + 8], idx, axis=0) for q in range(nq - 1, -1, -1)], axis=0)

    def p2_body(i, carry):
        t0 = i * NTB

        def ytile(c, odd):
            ng = 15 - odd
            cols = []
            for tt in range(NTB):
                rows = [ZS[c, t0 + tt, pl.ds(16 * g + 8 * odd, 8), :] for g in range(ng)]
                rows.append(jnp.zeros((128 - 8 * ng, 128), f32))
                cols.append(jnp.concatenate(rows, axis=0).astype(bf16))
            return jnp.concatenate(cols, axis=1)
        Ce = jnp.dot(GS[0], ytile(0, 0), preferred_element_type=f32)
        Se = jnp.dot(GS[1], ytile(1, 0), preferred_element_type=f32)
        Co = jnp.dot(GS[2], ytile(0, 1), preferred_element_type=f32)
        So = jnp.dot(GS[3], ytile(1, 1), preferred_element_type=f32)
        pp = Ce + Co
        mm = Ce - Co
        qq = Se + So
        rr = So - Se
        y = jnp.concatenate([mm + rr, revrows(pp + qq), pp - qq, revrows(mm - rr)], axis=0)
        xw = jnp.concatenate([XS[t0 + tt] for tt in range(NTB)], axis=1)
        h = (xw.astype(f32) + y).astype(bf16).astype(f32)
        mu = jnp.mean(h, axis=0, keepdims=True)
        hc = h - mu
        var = jnp.mean(hc * hc, axis=0, keepdims=True)
        a = (hc * jax.lax.rsqrt(var + EPS)).astype(bf16)
        at = a.T
        acc = h
        for fch in range(F // FC):
            sl = slice(fch * FC, (fch + 1) * FC)
            g = jnp.dot(at, WG[:, sl], preferred_element_type=f32)
            u = jnp.dot(at, WU[:, sl], preferred_element_type=f32)
            hh = (g * u).astype(bf16)
            acc = acc + jax.lax.dot_general(WD[:, sl], hh, NTDIMS, preferred_element_type=f32)
        off = pl.multiple_of(i * BM, BM)
        OS[:, pl.ds(off, BM)] = acc.astype(bf16)
        pltpu.make_async_copy(OS.at[:, pl.ds(off, BM)], o_hbm.at[:, pl.ds(off, BM)], sem_o.at[i]).start()
        return carry
    jax.lax.fori_loop(0, S // BM, p2_body, 0)
    for i in range(S // BM):
        pltpu.make_async_copy(OS.at[:, pl.ds(i * BM, BM)], o_hbm.at[:, pl.ds(i * BM, BM)], sem_o.at[i]).wait()


def build(interpret=False):
    def fn(A_x, A_w_r, A_w_i, B_x, B_w_gate, B_w_up, B_w_down):
        Ft, G, M = _tables()
        xt = jnp.transpose(A_x, (0, 2, 1)).reshape(D, S)
        any_spec = pl.BlockSpec(memory_space=pl.ANY)
        out = pl.pallas_call(
            _kernel,
            out_shape=jax.ShapeDtypeStruct((D, S), bf16),
            in_specs=[any_spec] * 9,
            out_specs=any_spec,
            scratch_shapes=[
                pltpu.VMEM((16, D, 128), bf16),
                pltpu.VMEM((2, 16, K, 128), bf16),
                pltpu.VMEM((2, 16, 128, 128), f32),
                pltpu.VMEM((2, 16, 120, 128), f32),
                pltpu.VMEM((2, 16, 232, 128), f32),
                pltpu.VMEM((16, 464, 128), bf16),
                pltpu.VMEM((4, 128, 128), bf16),
                pltpu.VMEM((4, 112, 128), bf16),
                pltpu.VMEM((16, 2, 128, 128), bf16),
                pltpu.VMEM((D, F), bf16),
                pltpu.VMEM((D, F), bf16),
                pltpu.VMEM((D, F), bf16),
                pltpu.VMEM((D, S), bf16),
                pltpu.SemaphoreType.DMA((16,)),
                pltpu.SemaphoreType.DMA((2, 16)),
                pltpu.SemaphoreType.DMA((3,)),
                pltpu.SemaphoreType.DMA((3,)),
                pltpu.SemaphoreType.DMA((S // BM,)),
            ],
            compiler_params=pltpu.CompilerParams(vmem_limit_bytes=100 * 2**20),
            interpret=(pltpu.InterpretParams() if interpret else False),
        )(xt, A_w_r.T, A_w_i.T, B_w_gate, B_w_up, B_w_down.T, jnp.asarray(Ft), jnp.asarray(G), jnp.asarray(M))
        return jnp.transpose(out.reshape(1, D, S), (0, 2, 1))
    return jax.jit(fn)


_forward = build()


@jax.jit
def pallas_sequential_preLN__spectral_gfnet__glu_gated_bilinear__prompt_kernel(
    A_x: jax.Array,
    A_w_r: jax.Array,
    A_w_i: jax.Array,
    B_x: jax.Array,
    B_w_gate: jax.Array,
    B_w_up: jax.Array,
    B_w_down: jax.Array,
):
    return _forward(A_x, A_w_r, A_w_i, B_x, B_w_gate, B_w_up, B_w_down)
```

```python
import numpy as np
import jax
import jax.numpy as jnp
import jax.experimental.pallas as pl
import jax.experimental.pallas.tpu as pltpu

S, D, F, K = 2048, 448, 1792, 225
EPS = 1e-5
bf16, f32, u32 = jnp.bfloat16, jnp.float32, jnp.uint32
NTDIMS = (((1,), (1,)), ((), ()))
NG = 29
WPITCH = 17


def _pack_rows(a):
    import ml_dtypes
    b = a.astype(ml_dtypes.bfloat16).view(np.uint16).astype(np.uint32)
    return b[..., 0::2, :] | (b[..., 1::2, :] << 16)


def _tables():
    th = 2 * np.pi / D
    nu = np.arange(112) + 0.5
    n = []
    for v in range(7):
        n += [16 * v + 2 * i for i in range(8)] + [16 * v + 2 * i + 1 for i in range(8)]
    nuf = np.array(n) + 0.5
    kE = 2 * np.arange(113)
    kO = 2 * np.arange(112) + 1
    Ft = np.zeros((4, 128, 128))
    Ft[0, :113, :112] = np.cos(np.outer(kE, nuf) * th)
    Ft[0, 112, :] = 0
    Ft[1, :113, :112] = -np.sin(np.outer(kE, nuf) * th)
    Ft[1, 0, :] = 0
    Ft[2, :112, :112] = np.cos(np.outer(kO, nuf) * th)
    Ft[3, :112, :112] = -np.sin(np.outer(kO, nuf) * th)
    cE = np.full(113, 2.0)
    cE[0] = 1
    cE[112] = 1
    sc = 1.0 / (D * S)
    G = np.zeros((4, 112, 128))
    gce = np.cos(np.outer(nu, kE) * th)
    gce[:, 112] = 0
    gse = np.sin(np.outer(nu, kE) * th)
    gse[:, 0] = 0
    G[0, :, :113] = gce * cE * sc
    G[1, :, :113] = gse * cE * sc
    G[2, :, :112] = np.cos(np.outer(nu, kO) * th) * 2 * sc
    G[3, :, :112] = np.sin(np.outer(nu, kO) * th) * 2 * sc
    a = np.arange(128)
    ph = -2 * np.pi * (np.outer(a, a) % 128) / 128
    base = np.zeros((2 * 128 + 32, 128), np.float32)
    base[0:128] = np.cos(ph)
    base[128:256] = np.sin(ph)
    d = np.arange(16)
    tw = -2 * np.pi * np.outer(d, a) / S
    base[256:272] = np.cos(tw)
    base[272:288] = np.sin(tw)
    return _pack_rows(Ft), _pack_rows(G), base


class Sg:
    __slots__ = ("v", "s")

    def __init__(self, v, s=1):
        self.v, self.s = v, s

    def __neg__(self):
        return Sg(self.v, -self.s)

    def __add__(self, o):
        if self.s == o.s:
            return Sg(self.v + o.v, self.s)
        if self.s > 0:
            return Sg(self.v - o.v, 1)
        return Sg(o.v - self.v, 1)

    def __sub__(self, o):
        return self + (-o)

    def scale(self, c):
        return Sg(self.v * np.float32(c * self.s), 1)

    def val(self):
        return self.v if self.s > 0 else -self.v


def _dft4(x, sgn):
    (r0, i0), (r1, i1), (r2, i2), (r3, i3) = x
    t0 = (r0 + r2, i0 + i2)
    t1 = (r0 - r2, i0 - i2)
    t2 = (r1 + r3, i1 + i3)
    t3 = (r1 - r3, i1 - i3)
    X0 = (t0[0] + t2[0], t0[1] + t2[1])
    X2 = (t0[0] - t2[0], t0[1] - t2[1])
    XA = (t1[0] + t3[1], t1[1] - t3[0])
    XB = (t1[0] - t3[1], t1[1] + t3[0])
    if sgn < 0:
        return [X0, XA, X2, XB]
    return [X0, XB, X2, XA]


def _tw16(z, e, sgn):
    r, i = z
    e = e % 16
    if e == 0:
        return z
    if e == 4:
        return (i, -r) if sgn < 0 else (-i, r)
    h = float(np.sqrt(0.5))
    if e in (2, 6):
        c = h if e == 2 else -h
        s = h * sgn
        re = (r if c > 0 else -r) - (i if s > 0 else -i)
        im = (r if s > 0 else -r) + (i if c > 0 else -i)
        return (re.scale(h), im.scale(h))
    c = float(np.cos(2 * np.pi * e / 16))
    s = float(sgn * np.sin(2 * np.pi * e / 16))
    return (r.scale(c) - i.scale(s), r.scale(s) + i.scale(c))


def _fft16(x, sgn):
    x = [(Sg(r), Sg(i)) for r, i in x]
    U = [_dft4([x[4 * b1 + b0] for b1 in range(4)], sgn) for b0 in range(4)]
    V = [[_tw16(U[b0][d0], d0 * b0, sgn) for d0 in range(4)] for b0 in range(4)]
    out = [None] * 16
    for d0 in range(4):
        X = _dft4([V[b0][d0] for b0 in range(4)], sgn)
        for d1 in range(4):
            out[d0 + 4 * d1] = (X[d1][0].val(), X[d1][1].val())
    return out


def _unpack(u):
    lo = pltpu.bitcast(u << 16, f32)
    hi = pltpu.bitcast(u & np.uint32(0xFFFF0000), f32)
    return lo, hi


def _asbf(u):
    return pltpu.bitcast(u, bf16)


def _make_kernel(BM, FC, NPASS, XGROUPS, CSPLIT, unroll_b, WSTART, WPRI):
    def _kernel(x_hbm, wr_hbm, wi_hbm, wg_hbm, wu_hbm, wd_hbm, f_hbm, g_hbm, b_hbm, o_hbm,
                XS, WS, WT, WP, ZS, TS, FS, GS, BS, MS, WG, WU, WD, OS, AT, HS, ACC,
                sem_x, sem_w, sem_t, sem_m, sem_o):
        ct = [pltpu.make_async_copy(b_hbm, BS, sem_t.at[0]),
              pltpu.make_async_copy(f_hbm, FS, sem_t.at[1]),
              pltpu.make_async_copy(g_hbm, GS, sem_t.at[2])]
        cx = [pltpu.make_async_copy(x_hbm.at[:, pl.ds(t * 128, 128)], XS.at[t], sem_x.at[t]) for t in range(16)]
        cw = [[pltpu.make_async_copy(w.at[:, pl.ds(t * 128, 128)], WS.at[c, t], sem_w.at[c, t]) for t in range(16)]
              for c, w in enumerate((wr_hbm, wi_hbm))]
        NCH = F // FC
        cm = [[pltpu.make_async_copy(a.at[:, pl.ds(j * FC, FC)], b.at[:, pl.ds(j * FC, FC)], sem_m.at[j, i])
               for i, (a, b) in enumerate(((wg_hbm, WG), (wu_hbm, WU), (wd_hbm, WD)))] for j in range(NCH)]
        ct[0].start(priority=0)
        ct[1].start(priority=0)
        for c in cx:
            c.start(priority=1)

        row8 = jax.lax.broadcasted_iota(jnp.int32, (8, 128), 0)
        rev8 = 7 - row8

        ct[0].wait()
        ct[1].wait()
        for d in range(16):
            twr = jnp.broadcast_to(BS[256 + d:257 + d, :], (8, 128))
            twi = jnp.broadcast_to(BS[272 + d:273 + d, :], (8, 128))
            for q in range(8):
                fre = BS[16 * q:16 * q + 8, :]
                fro = BS[16 * q + 8:16 * q + 16, :]
                fie = BS[128 + 16 * q:128 + 16 * q + 8, :]
                fio = BS[128 + 16 * q + 8:128 + 16 * q + 16, :]
                if d == 0:
                    mre, mro, mie, mio = fre, fro, fie, fio
                else:
                    mre = fre * twr - fie * twi
                    mro = fro * twr - fio * twi
                    mie = fre * twi + fie * twr
                    mio = fro * twi + fio * twr
                MS[d, 0, pl.ds(16 * q, 16), :] = jnp.concatenate([mre, mro], axis=0).astype(bf16)
                MS[d, 1, pl.ds(16 * q, 16), :] = jnp.concatenate([mie, mio], axis=0).astype(bf16)

        def p1a(t):
            def ld(v, reverse):
                u = pltpu.bitcast(XS[t, pl.ds(16 * v, 16), :], u32)
                if reverse:
                    u = jnp.take_along_axis(u, rev8, axis=0)
                return _unpack(u)
            Ree, Ro, Ie, Io = [], [], [], []
            sq = None
            for v in range(7):
                Al, Ah = ld(v, False)
                Bl, Bh = ld(27 - v, True)
                Cl, Ch = ld(13 - v, True)
                Dl, Dh = ld(14 + v, False)
                for (a, b, c, d) in ((Al, Bh, Ch, Dl), (Ah, Bl, Cl, Dh)):
                    p = a + b
                    q = c + d
                    r = a - b
                    s = d - c
                    ro, ie, io = q - p, s + r, s - r
                    Ree.append(q + p)
                    Ro.append(ro)
                    Ie.append(ie)
                    Io.append(io)
                    t2 = ro * ro + ie * ie + io * io
                    sq = t2 if sq is None else sq + t2
            tot = Ree[0]
            for z in Ree[1:]:
                tot = tot + z
            mean4 = jnp.sum(tot, axis=0, keepdims=True) * np.float32(4.0 / D)
            Ree = [z - mean4 for z in Ree]
            for z in Ree:
                sq = sq + z * z
            var = jnp.sum(sq, axis=0, keepdims=True) * np.float32(1.0 / (4 * D))
            rstd = jax.lax.rsqrt(var + EPS)
            zpad = jnp.zeros((16, 128), f32)
            for blk, lst in enumerate((Ree, Ie, Ro, Io)):
                data = jnp.concatenate(lst + [zpad], axis=0).astype(bf16)
                nrow = 64 if blk < 2 else 56
                z = jnp.dot(_asbf(FS[blk, 0:nrow, :]), data, preferred_element_type=f32) * rstd
                c = blk % 2
                odd = blk // 2
                for g in range(15 - odd):
                    ZS[c, t, pl.ds(16 * g + 8 * odd, 8), :] = z[8 * g:8 * g + 8, :]

        t = 0
        for gi, n in enumerate(XGROUPS):
            for tt in range(t, t + n):
                cx[tt].wait()
            if gi == WSTART:
                for tt in range(16):
                    cw[0][tt].start(priority=WPRI)
                    cw[1][tt].start(priority=WPRI)
            if gi == len(XGROUPS) - 1:
                ct[2].start(priority=1)
                for c in cm[0]:
                    c.start(priority=1)
            for tt in range(t, t + n):
                p1a(tt)
            t += n
        assert t == 16

        def s1(g):
            r0 = g * 8 if isinstance(g, int) else pl.multiple_of(g * 8, 8)
            x = [(ZS[0, b, pl.ds(r0, 8), :], ZS[1, b, pl.ds(r0, 8), :]) for b in range(16)]
            T = _fft16(x, -1)
            q0 = g * 16 if isinstance(g, int) else pl.multiple_of(g * 16, 16)
            for d in range(16):
                TS[d, pl.ds(q0, 16), :] = jnp.concatenate([T[d][0], T[d][1]], axis=0).astype(bf16)

        def s1_body(g, carry):
            s1(g)
            return carry
        if unroll_b:
            for g in range(NG):
                s1(g)
        else:
            jax.lax.fori_loop(0, NG, s1_body, 0)

        def t1(t, c):
            u = pltpu.bitcast(WS[c, t, 0:224, :], u32)
            w224 = pltpu.bitcast(WS[c, t, 224:225, :].astype(f32), u32) >> 16
            last = jnp.where(row8 == 0, jnp.broadcast_to(w224, (8, 128)), np.uint32(0))
            full = jnp.concatenate([u, last, jnp.zeros((8, 128), u32)], axis=0)
            ut = pltpu.bitcast(full, f32).T
            for q in range(8):
                WT[c, t, pl.ds(WPITCH * q, 16), :] = ut[16 * q:16 * q + 16, :]

        def t2(d, c):
            Gm = jnp.concatenate([WT[c, t, pl.ds(d, 8, stride=WPITCH), :] for t in range(16)], axis=0)
            WP[c, d] = Gm.T[0:120, :]

        def s2(d):
            lhs = TS[d]
            A = jax.lax.dot_general(lhs, MS[d, 0], NTDIMS, preferred_element_type=f32)
            B = jax.lax.dot_general(lhs, MS[d, 1], NTDIMS, preferred_element_type=f32)
            for gam in range(NG):
                ZS[0, d, pl.ds(8 * gam, 8), :] = A[16 * gam:16 * gam + 8] - B[16 * gam + 8:16 * gam + 16]
                ZS[1, d, pl.ds(8 * gam, 8), :] = B[16 * gam:16 * gam + 8] + A[16 * gam + 8:16 * gam + 16]

        def s2i(d):
            P = []
            for gg in range(15):
                wrl, wrh = _unpack(pltpu.bitcast(WP[0, d, pl.ds(8 * gg, 8), :], u32))
                wil, wih = _unpack(pltpu.bitcast(WP[1, d, pl.ds(8 * gg, 8), :], u32))
                for odd in range(2):
                    gam = 2 * gg + odd
                    if gam >= NG:
                        continue
                    wr_, wi_ = (wrl, wil) if odd == 0 else (wrh, wih)
                    zr = ZS[0, d, pl.ds(8 * gam, 8), :]
                    zi = ZS[1, d, pl.ds(8 * gam, 8), :]
                    P.append(zr * wr_ - zi * wi_)
                    P.append(zr * wi_ + zi * wr_)
            Pb = jnp.concatenate(P, axis=0).astype(bf16)
            A2 = jnp.dot(Pb, MS[d, 0], preferred_element_type=f32)
            B2 = jnp.dot(Pb, MS[d, 1], preferred_element_type=f32)
            for gam in range(NG):
                ZS[0, d, pl.ds(8 * gam, 8), :] = A2[16 * gam:16 * gam + 8] + B2[16 * gam + 8:16 * gam + 16]
                ZS[1, d, pl.ds(8 * gam, 8), :] = A2[16 * gam + 8:16 * gam + 16] - B2[16 * gam:16 * gam + 8]

        for d in range(CSPLIT):
            s2(d)
        for t in range(16):
            cw[0][t].wait()
            cw[1][t].wait()
        rest = list(range(CSPLIT, 16))
        t1jobs = [(t, c) for t in range(16) for c in range(2)]
        per = -(-len(t1jobs) // max(len(rest), 1))
        for i, d in enumerate(rest):
            for (t, c) in t1jobs[i * per:(i + 1) * per]:
                t1(t, c)
            s2(d)
        if not rest:
            for (t, c) in t1jobs:
                t1(t, c)
        t2(0, 0)
        t2(0, 1)
        for d in range(16):
            if d + 1 < 16:
                t2(d + 1, 0)
                t2(d + 1, 1)
            s2i(d)

        def s1i(g):
            r0 = g * 8 if isinstance(g, int) else pl.multiple_of(g * 8, 8)
            x = [(ZS[0, b, pl.ds(r0, 8), :], ZS[1, b, pl.ds(r0, 8), :]) for b in range(16)]
            Y = _fft16(x, +1)
            for b in range(16):
                ZS[0, b, pl.ds(r0, 8), :] = Y[b][0]
                ZS[1, b, pl.ds(r0, 8), :] = Y[b][1]

        def s1i_body(g, carry):
            s1i(g)
            return carry
        if unroll_b:
            for g in range(NG):
                s1i(g)
        else:
            jax.lax.fori_loop(0, NG, s1i_body, 0)

        ct[2].wait()
        NTB = BM // 128
        NB = S // BM

        def revrows(z):
            nq = z.shape[0] // 8
            idx = 7 - jax.lax.broadcasted_iota(jnp.int32, (8, z.shape[1]), 0)
            return jnp.concatenate(
                [jnp.take_along_axis(z[8 * q:8 * q + 8], idx, axis=0) for q in range(nq - 1, -1, -1)], axis=0)

        def prep(i):
            t0 = i * NTB

            def ytile(c, odd):
                ng = 15 - odd
                cols = []
                zero = jnp.zeros((8, 128), f32)
                for tt in range(NTB):
                    rows = [ZS[c, t0 + tt, pl.ds(16 * g + 8 * odd, 8), :] for g in range(ng)]
                    rows += [zero] * (16 - ng)
                    cols.append(jnp.concatenate(rows, axis=0))
                return jnp.concatenate(cols, axis=1).astype(bf16)
            Ce = jnp.dot(_asbf(GS[0]), ytile(0, 0), preferred_element_type=f32)
            Se = jnp.dot(_asbf(GS[1]), ytile(1, 0), preferred_element_type=f32)
            Co = jnp.dot(_asbf(GS[2]), ytile(0, 1), preferred_element_type=f32)
            So = jnp.dot(_asbf(GS[3]), ytile(1, 1), preferred_element_type=f32)
            pp = Ce + Co
            mm = Ce - Co
            qq = Se + So
            rr = So - Se
            y = jnp.concatenate([mm + rr, revrows(pp + qq), pp - qq, revrows(mm - rr)], axis=0)
            xw = jnp.concatenate([XS[t0 + tt] for tt in range(NTB)], axis=1)
            h = (xw.astype(f32) + y).astype(bf16).astype(f32)
            mu = jnp.mean(h, axis=0, keepdims=True)
            hc = h - mu
            var = jnp.mean(hc * hc, axis=0, keepdims=True)
            a = (hc * jax.lax.rsqrt(var + EPS)).astype(bf16)
            return h, a.T

        def mlp(at, acc, chunks):
            for fch in chunks:
                sl = slice(fch * FC, (fch + 1) * FC)
                g = jnp.dot(at, WG[:, sl], preferred_element_type=f32)
                u = jnp.dot(at, WU[:, sl], preferred_element_type=f32)
                hh = (g * u).astype(bf16)
                acc = acc + jax.lax.dot_general(WD[:, sl], hh, NTDIMS, preferred_element_type=f32)
            return acc

        def out_copy(i):
            off = i * BM if isinstance(i, int) else pl.multiple_of(i * BM, BM)
            return pltpu.make_async_copy(OS.at[:, pl.ds(off, BM)], o_hbm.at[:, pl.ds(off, BM)], sem_o.at[i])

        if NPASS == 1:
            for j in range(1, NCH):
                for c in cm[j]:
                    c.start()
            for j in range(NCH):
                for c in cm[j]:
                    c.wait()

            def p2_body(i, carry):
                h, at = prep(i)
                acc = mlp(at, h, range(NCH))
                off = pl.multiple_of(i * BM, BM)
                OS[:, pl.ds(off, BM)] = acc.astype(bf16)
                out_copy(i).start()
                return carry
            jax.lax.fori_loop(0, NB, p2_body, 0)
        else:
            for j in range(NCH):
                for c in cm[j]:
                    c.wait()
                if j + 1 < NCH:
                    for c in cm[j + 1]:
                        c.start()

                def body(i, carry, j=j):
                    off = pl.multiple_of(i * BM, BM)
                    if j == 0:
                        h, at = prep(i)
                        AT[i] = at
                    else:
                        h = ACC[:, pl.ds(off, BM)]
                        at = AT[i]
                    acc = mlp(at, h, [j])
                    if j == NCH - 1:
                        OS[:, pl.ds(off, BM)] = acc.astype(bf16)
                        out_copy(i).start()
                    else:
                        ACC[:, pl.ds(off, BM)] = acc
                    return carry
                jax.lax.fori_loop(0, NB, body, 0)
        for i in range(NB):
            out_copy(i).wait()
    return _kernel


def build(interpret=False, BM=512, FC=896, NPASS=2, XGROUPS=(4, 4, 4, 4), CSPLIT=8, unroll_b=True, WSTART=2, WPRI=1):
    def fn(A_x, A_w_r, A_w_i, B_x, B_w_gate, B_w_up, B_w_down):
        Ft, G, base = _tables()
        xt = jnp.transpose(A_x, (0, 2, 1)).reshape(D, S)
        any_spec = pl.BlockSpec(memory_space=pl.ANY)
        out = pl.pallas_call(
            _make_kernel(BM, FC, NPASS, XGROUPS, CSPLIT, unroll_b, WSTART, WPRI),
            out_shape=jax.ShapeDtypeStruct((D, S), bf16),
            in_specs=[any_spec] * 9,
            out_specs=any_spec,
            scratch_shapes=[
                pltpu.VMEM((16, D, 128), bf16),
                pltpu.VMEM((2, 16, K, 128), bf16),
                pltpu.VMEM((2, 16, 8 * WPITCH, 128), f32),
                pltpu.VMEM((2, 16, 120, 128), f32),
                pltpu.VMEM((2, 16, 8 * NG, 128), f32),
                pltpu.VMEM((16, 16 * NG, 128), bf16),
                pltpu.VMEM((4, 64, 128), u32),
                pltpu.VMEM((4, 56, 128), u32),
                pltpu.VMEM((288, 128), f32),
                pltpu.VMEM((16, 2, 128, 128), bf16),
                pltpu.VMEM((D, F), bf16),
                pltpu.VMEM((D, F), bf16),
                pltpu.VMEM((D, F), bf16),
                pltpu.VMEM((D, S), bf16),
                pltpu.VMEM((S // BM, BM, D), bf16),
                pltpu.VMEM((8, 128), f32),
                pltpu.VMEM((D, S), f32),
                pltpu.SemaphoreType.DMA((16,)),
                pltpu.SemaphoreType.DMA((2, 16)),
                pltpu.SemaphoreType.DMA((3,)),
                pltpu.SemaphoreType.DMA((F // FC, 3)),
                pltpu.SemaphoreType.DMA((S // BM,)),
            ],
            compiler_params=pltpu.CompilerParams(vmem_limit_bytes=100 * 2**20),
            interpret=(pltpu.InterpretParams() if interpret else False),
        )(xt, A_w_r.T, A_w_i.T, B_w_gate, B_w_up, B_w_down.T, jnp.asarray(Ft), jnp.asarray(G), jnp.asarray(base))
        return jnp.transpose(out.reshape(1, D, S), (0, 2, 1))
    return jax.jit(fn)


_forward = build()


@jax.jit
def pallas_sequential_preLN__spectral_gfnet__glu_gated_bilinear__prompt_kernel(
    A_x: jax.Array,
    A_w_r: jax.Array,
    A_w_i: jax.Array,
    B_x: jax.Array,
    B_w_gate: jax.Array,
    B_w_up: jax.Array,
    B_w_down: jax.Array,
):
    return _forward(A_x, A_w_r, A_w_i, B_x, B_w_gate, B_w_up, B_w_down)
```

```python
import numpy as np
import jax
import jax.numpy as jnp
import jax.experimental.pallas as pl
import jax.experimental.pallas.tpu as pltpu

S, D, F, K = 2048, 448, 1792, 225
EPS = 1e-5
bf16, f32, u32 = jnp.bfloat16, jnp.float32, jnp.uint32
NTDIMS = (((1,), (1,)), ((), ()))
NG = 29
WPITCH = 17
NB = 4
BM = S // NB


def _pack_rows(a):
    import ml_dtypes
    b = a.astype(ml_dtypes.bfloat16).view(np.uint16).astype(np.uint32)
    return b[..., 0::2, :] | (b[..., 1::2, :] << 16)


def _tables():
    th = 2 * np.pi / D
    nu = np.arange(112) + 0.5
    n = []
    for v in range(7):
        n += [16 * v + 2 * i for i in range(8)] + [16 * v + 2 * i + 1 for i in range(8)]
    nuf = np.array(n) + 0.5
    kE = 2 * np.arange(113)
    kO = 2 * np.arange(112) + 1
    Ft = np.zeros((4, 128, 128))
    Ft[0, :113, :112] = np.cos(np.outer(kE, nuf) * th)
    Ft[0, 112, :] = 0
    Ft[1, :113, :112] = -np.sin(np.outer(kE, nuf) * th)
    Ft[1, 0, :] = 0
    Ft[2, :112, :112] = np.cos(np.outer(kO, nuf) * th)
    Ft[3, :112, :112] = -np.sin(np.outer(kO, nuf) * th)
    cE = np.full(113, 2.0)
    cE[0] = 1
    cE[112] = 1
    sc = 1.0 / (D * S)
    G = np.zeros((4, 112, 128))
    gce = np.cos(np.outer(nu, kE) * th)
    gce[:, 112] = 0
    gse = np.sin(np.outer(nu, kE) * th)
    gse[:, 0] = 0
    G[0, :, :113] = gce * cE * sc
    G[1, :, :113] = gse * cE * sc
    G[2, :, :112] = np.cos(np.outer(nu, kO) * th) * 2 * sc
    G[3, :, :112] = np.sin(np.outer(nu, kO) * th) * 2 * sc
    a = np.arange(128)
    ph = -2 * np.pi * (np.outer(a, a) % 128) / 128
    base = np.zeros((2 * 128 + 32, 128), np.float32)
    base[0:128] = np.cos(ph)
    base[128:256] = np.sin(ph)
    d = np.arange(16)
    tw = -2 * np.pi * np.outer(d, a) / S
    base[256:272] = np.cos(tw)
    base[272:288] = np.sin(tw)
    return _pack_rows(Ft), _pack_rows(G), base


class Sg:
    __slots__ = ("v", "s")

    def __init__(self, v, s=1):
        self.v, self.s = v, s

    def __neg__(self):
        return Sg(self.v, -self.s)

    def __add__(self, o):
        if self.s == o.s:
            return Sg(self.v + o.v, self.s)
        if self.s > 0:
            return Sg(self.v - o.v, 1)
        return Sg(o.v - self.v, 1)

    def __sub__(self, o):
        return self + (-o)

    def scale(self, c):
        return Sg(self.v * np.float32(c * self.s), 1)

    def val(self):
        return self.v if self.s > 0 else -self.v


def _dft4_finish(t0, t1, t2, t3, sgn):
    X0 = (t0[0] + t2[0], t0[1] + t2[1])
    X2 = (t0[0] - t2[0], t0[1] - t2[1])
    XA = (t1[0] + t3[1], t1[1] - t3[0])
    XB = (t1[0] - t3[1], t1[1] + t3[0])
    if sgn < 0:
        return [X0, XA, X2, XB]
    return [X0, XB, X2, XA]


def _dft4(x, sgn):
    (r0, i0), (r1, i1), (r2, i2), (r3, i3) = x
    return _dft4_finish((r0 + r2, i0 + i2), (r0 - r2, i0 - i2), (r1 + r3, i1 + i3), (r1 - r3, i1 - i3), sgn)


def _tw16(z, e, sgn):
    r, i = z
    e = e % 16
    if e == 0:
        return z
    if e == 4:
        return (i, -r) if sgn < 0 else (-i, r)
    h = float(np.sqrt(0.5))
    if e in (2, 6):
        c = h if e == 2 else -h
        s = h * sgn
        re = (r if c > 0 else -r) - (i if s > 0 else -i)
        im = (r if s > 0 else -r) + (i if c > 0 else -i)
        return (re.scale(h), im.scale(h))
    c = float(np.cos(2 * np.pi * e / 16))
    s = float(sgn * np.sin(2 * np.pi * e / 16))
    return (r.scale(c) - i.scale(s), r.scale(s) + i.scale(c))


def _sg(z):
    return (Sg(z[0]), Sg(z[1]))


def _bf_lo(u):
    return pltpu.bitcast(u << 16, f32)


def _bf_hi(u):
    return pltpu.bitcast(u & np.uint32(0xFFFF0000), f32)


def _asbf(u):
    return pltpu.bitcast(u, bf16)


import contextlib


def _make_kernel(FC, WWAITS, WSTART, P0MODE, T2AHEAD, XPRI, MGEN, MGEN0, SCOPES, EORDER, SPLIT0, SPLITL):
    def sc(name):
        return jax.named_scope(name) if SCOPES else contextlib.nullcontext()

    NCH = F // FC

    def _kernel(x_hbm, wr_hbm, wi_hbm, wg_hbm, wu_hbm, wd_hbm, f_hbm, g_hbm, b_hbm, o_hbm,
                XS, WS, WT, WP, VF, FP, TH, TE, VI, YB, FS, GS, BS, MS, WG, WU, WD, OS, AT, ACC,
                sem_x, sem_w, sem_t, sem_m, sem_o):
        wgrp = {t: gi for gi, (_, a, b) in enumerate(WWAITS) for t in range(a, b)}
        ct = [pltpu.make_async_copy(b_hbm, BS, sem_t.at[0]),
              pltpu.make_async_copy(f_hbm, FS, sem_t.at[0]),
              pltpu.make_async_copy(g_hbm, GS, sem_t.at[1])]
        cx = [pltpu.make_async_copy(x_hbm.at[:, pl.ds(t * 128, 128)], XS.at[t], sem_x.at[t % 4]) for t in range(16)]
        cw = [[pltpu.make_async_copy(w.at[:, pl.ds(t * 128, 128)], WS.at[c, t], sem_w.at[wgrp[t]]) for t in range(16)]
              for c, w in enumerate((wr_hbm, wi_hbm))]
        cm = [[pltpu.make_async_copy(a.at[:, pl.ds(j * FC, FC)], b.at[:, pl.ds(j * FC, FC)], sem_m.at[j])
               for i, (a, b) in enumerate(((wg_hbm, WG), (wu_hbm, WU), (wd_hbm, WD)))] for j in range(NCH)]
        ct[0].start(priority=0)
        ct[1].start(priority=0)
        for j in range(4):
            for b1 in range(4):
                cx[j + 4 * b1].start(priority=XPRI[j])

        row8 = jax.lax.broadcasted_iota(jnp.int32, (8, 128), 0)
        rev8 = 7 - row8

        with sc("w_tab"):
            ct[0].wait()
            ct[1].wait()

        def gen_m(d):
            twr = jnp.broadcast_to(BS[256 + d:257 + d, :], (8, 128))
            twi = jnp.broadcast_to(BS[272 + d:273 + d, :], (8, 128))
            for q in range(8):
                fre = BS[16 * q:16 * q + 8, :]
                fro = BS[16 * q + 8:16 * q + 16, :]
                fie = BS[128 + 16 * q:128 + 16 * q + 8, :]
                fio = BS[128 + 16 * q + 8:128 + 16 * q + 16, :]
                if d == 0:
                    mre, mro, mie, mio = fre, fro, fie, fio
                else:
                    mre = fre * twr - fie * twi
                    mro = fro * twr - fio * twi
                    mie = fre * twi + fie * twr
                    mio = fro * twi + fio * twr
                MS[d, 0, pl.ds(16 * q, 16), :] = jnp.concatenate([mre, mro], axis=0).astype(bf16)
                MS[d, 1, pl.ds(16 * q, 16), :] = jnp.concatenate([mie, mio], axis=0).astype(bf16)

        if MGEN == 0:
            for d in range(16):
                gen_m(d)

        def fold_tile(t):
            def ld(v, reverse):
                u = pltpu.bitcast(XS[t, pl.ds(16 * v, 16), :], u32)
                if reverse:
                    u = jnp.take_along_axis(u, rev8, axis=0)
                return _bf_lo(u), _bf_hi(u)
            Ree, Ro, Ie, Io = [], [], [], []
            sq = None
            for v in range(7):
                Al, Ah = ld(v, False)
                Bl, Bh = ld(27 - v, True)
                Cl, Ch = ld(13 - v, True)
                Dl, Dh = ld(14 + v, False)
                for (a, b, c, d) in ((Al, Bh, Ch, Dl), (Ah, Bl, Cl, Dh)):
                    p = a + b
                    q = c + d
                    r = a - b
                    s = d - c
                    ro, ie, io = q - p, s + r, s - r
                    Ree.append(q + p)
                    Ro.append(ro)
                    Ie.append(ie)
                    Io.append(io)
                    t2 = ro * ro + ie * ie + io * io
                    sq = t2 if sq is None else sq + t2
            tot = Ree[0]
            for z in Ree[1:]:
                tot = tot + z
            mean4 = jnp.sum(tot, axis=0, keepdims=True) * np.float32(4.0 / D)
            Ree = [z - mean4 for z in Ree]
            for z in Ree:
                sq = sq + z * z
            var = jnp.sum(sq, axis=0, keepdims=True) * np.float32(1.0 / (4 * D))
            rstd = jax.lax.rsqrt(var + EPS)
            return (Ree, Ie, Ro, Io), rstd

        def stage_a(j):
            for rnd in range(2):
                parts = [fold_tile(j + 4 * b1) for b1 in (rnd, rnd + 2)]
                rstd = jnp.concatenate([p[1] for p in parts], axis=1)
                zpad = jnp.zeros((16, 256), f32)
                for odd in range(2):
                    z = []
                    for blk in (2 * odd, 2 * odd + 1):
                        rows = [jnp.concatenate([parts[i][0][blk][v] for i in range(2)], axis=1) for v in range(14)]
                        data = jnp.concatenate(rows + [zpad], axis=0).astype(bf16)
                        nrow = 56 if odd else 64
                        z.append(jnp.dot(_asbf(FS[blk, 0:nrow, :]), data, preferred_element_type=f32))
                    for g in range(15 - odd):
                        rs = pl.ds(16 * g + 8 * odd, 8)
                        zr = z[0][8 * g:8 * g + 8, :] * rstd
                        zi = z[1][8 * g:8 * g + 8, :] * rstd
                        xa = (Sg(zr[:, 0:128]), Sg(zi[:, 0:128]))
                        xb = (Sg(zr[:, 128:256]), Sg(zi[:, 128:256]))
                        ta = (xa[0] + xb[0], xa[1] + xb[1])
                        tb = (xa[0] - xb[0], xa[1] - xb[1])
                        if rnd == 0:
                            TH[0, 0, rs, :] = ta[0].val()
                            TH[1, 0, rs, :] = ta[1].val()
                            TH[0, 1, rs, :] = tb[0].val()
                            TH[1, 1, rs, :] = tb[1].val()
                        else:
                            t0 = (Sg(TH[0, 0, rs, :]), Sg(TH[1, 0, rs, :]))
                            t1_ = (Sg(TH[0, 1, rs, :]), Sg(TH[1, 1, rs, :]))
                            U = _dft4_finish(t0, t1_, ta, tb, -1)
                            for d0 in range(4):
                                vr, vi = _tw16(U[d0], d0 * j, -1)
                                VF[0, j, d0, rs, :] = vr.val()
                                VF[1, j, d0, rs, :] = vi.val()

        for j in range(4):
            with sc("w_x"):
                for b1 in range(4):
                    cx[j + 4 * b1].wait()
            if j == WSTART:
                for t in range(16):
                    cw[0][t].start(priority=1)
                    cw[1][t].start(priority=1)
            if j == 3:
                ct[2].start(priority=1)
                for c in cm[0]:
                    c.start(priority=1)
            stage_a(j)
            if MGEN and j == MGEN0:
                gen_m(0)
                gen_m(8)

        def t1(t, c):
            u = pltpu.bitcast(WS[c, t, 0:224, :], u32)
            w224 = pltpu.bitcast(WS[c, t, 224:225, :].astype(f32), u32) >> 16
            last = jnp.where(row8 == 0, jnp.broadcast_to(w224, (8, 128)), np.uint32(0))
            full = jnp.concatenate([u, last, jnp.zeros((8, 128), u32)], axis=0)
            ut = pltpu.bitcast(full, f32).T
            for q in range(8):
                WT[c, t, pl.ds(WPITCH * q, 16), :] = ut[16 * q:16 * q + 16, :]

        def wslot(d):
            return d

        def t2(d, c):
            Gm = jnp.concatenate([WT[c, t, pl.ds(d, 8, stride=WPITCH), :] for t in range(16)], axis=0)
            WP[c, wslot(d)] = Gm.T[0:120, :]

        def stage_c(d0, half):
            la, lb = [], []
            for gam in range(NG):
                x = [(Sg(VF[0, b0, d0, pl.ds(8 * gam, 8), :]), Sg(VF[1, b0, d0, pl.ds(8 * gam, 8), :])) for b0 in range(4)]
                if half == 0:
                    t0 = (x[0][0] + x[2][0], x[0][1] + x[2][1])
                    t2_ = (x[1][0] + x[3][0], x[1][1] + x[3][1])
                    Xa = (t0[0] + t2_[0], t0[1] + t2_[1])
                    Xb = (t0[0] - t2_[0], t0[1] - t2_[1])
                else:
                    t1_ = (x[0][0] - x[2][0], x[0][1] - x[2][1])
                    t3 = (x[1][0] - x[3][0], x[1][1] - x[3][1])
                    Xa = (t1_[0] + t3[1], t1_[1] - t3[0])
                    Xb = (t1_[0] - t3[1], t1_[1] + t3[0])
                la += [Xa[0].val(), Xa[1].val()]
                lb += [Xb[0].val(), Xb[1].val()]
            da = d0 + 4 * half
            for d, lst in ((da, la), (da + 8, lb)):
                lhs = jnp.concatenate(lst, axis=0).astype(bf16)
                A = jax.lax.dot_general(lhs, MS[d, 0], NTDIMS, preferred_element_type=f32)
                B = jax.lax.dot_general(lhs, MS[d, 1], NTDIMS, preferred_element_type=f32)
                for gam in range(NG):
                    r = 16 * gam
                    FP[0, d, pl.ds(8 * gam, 8), :] = A[r:r + 8] - B[r + 8:r + 16]
                    FP[1, d, pl.ds(8 * gam, 8), :] = B[r:r + 8] + A[r + 8:r + 16]

        passes = [(d0, half) for d0 in range(4) for half in range(2)]
        wwait = {p: (a, b) for (p, a, b) in WWAITS}
        pending, per = [], 0
        for p, (d0, half) in enumerate(passes):
            if p in wwait:
                a, b = wwait[p]
                with sc("w_w"):
                    for t in range(a, b):
                        cw[0][t].wait()
                        cw[1][t].wait()
                pending = [(t, c) for t in range(a, b) for c in range(2)]
                nxt = [q for q in sorted(wwait) if q > p]
                span = (nxt[0] if nxt else len(passes)) - p
                per = -(-len(pending) // span)
            for (t, c) in pending[:per]:
                t1(t, c)
            pending = pending[per:]
            if MGEN and p + 1 < len(passes):
                gen_m(passes[p + 1][0] + 4 * passes[p + 1][1])
                gen_m(passes[p + 1][0] + 4 * passes[p + 1][1] + 8)
            stage_c(d0, half)
        assert not pending

        def t2_val(d, c):
            Gm = jnp.concatenate([WT[c, t, pl.ds(d, 8, stride=WPITCH), :] for t in range(16)], axis=0)
            return pltpu.bitcast(Gm.T, u32)

        def w_mul(d):
            P = []
            if T2AHEAD < 0:
                wtr, wti = t2_val(d, 0), t2_val(d, 1)
            for gam in range(NG):
                gg, odd = gam // 2, gam % 2
                if T2AHEAD < 0:
                    wu_r = wtr[8 * gg:8 * gg + 8]
                    wu_i = wti[8 * gg:8 * gg + 8]
                else:
                    wu_r = pltpu.bitcast(WP[0, wslot(d), pl.ds(8 * gg, 8), :], u32)
                    wu_i = pltpu.bitcast(WP[1, wslot(d), pl.ds(8 * gg, 8), :], u32)
                wr_ = _bf_hi(wu_r) if odd else _bf_lo(wu_r)
                wi_ = _bf_hi(wu_i) if odd else _bf_lo(wu_i)
                zr = FP[0, d, pl.ds(8 * gam, 8), :]
                zi = FP[1, d, pl.ds(8 * gam, 8), :]
                P.append(zr * wr_ - zi * wi_)
                P.append(zr * wi_ + zi * wr_)
            Pb = jnp.concatenate(P, axis=0).astype(bf16)
            A2 = jnp.dot(Pb, MS[d, 0], preferred_element_type=f32)
            B2 = jnp.dot(Pb, MS[d, 1], preferred_element_type=f32)
            out = []
            for gam in range(NG):
                r = 16 * gam
                out.append((Sg(A2[r:r + 8] + B2[r + 8:r + 16]), Sg(A2[r + 8:r + 16] - B2[r:r + 8])))
            return out

        def stage_e(d0, half):
            da = d0 + 4 * half
            ua = w_mul(da)
            ub = w_mul(da + 8)
            for gam in range(NG):
                rs = pl.ds(8 * gam, 8)
                ta = (ua[gam][0] + ub[gam][0], ua[gam][1] + ub[gam][1])
                tb = (ua[gam][0] - ub[gam][0], ua[gam][1] - ub[gam][1])
                if half == 0:
                    TE[d0, 0, 0, rs, :] = ta[0].val()
                    TE[d0, 1, 0, rs, :] = ta[1].val()
                    TE[d0, 0, 1, rs, :] = tb[0].val()
                    TE[d0, 1, 1, rs, :] = tb[1].val()
                else:
                    t0 = (Sg(TE[d0, 0, 0, rs, :]), Sg(TE[d0, 1, 0, rs, :]))
                    t1_ = (Sg(TE[d0, 0, 1, rs, :]), Sg(TE[d0, 1, 1, rs, :]))
                    X = _dft4_finish(t0, t1_, ta, tb, +1)
                    for b0 in range(4):
                        vr, vi = _tw16(X[b0], d0 * b0, +1)
                        VI[0, b0, d0, rs, :] = vr.val()
                        VI[1, b0, d0, rs, :] = vi.val()

        if EORDER == 1:
            passes = [(d0, half) for half in range(2) for d0 in range(4)]
        elif EORDER == 2:
            passes = [(0, 0), (1, 0), (0, 1), (2, 0), (1, 1), (3, 0), (2, 1), (3, 1)]
        t2jobs = [[(d0 + 4 * half + 8 * s, c) for s in range(2) for c in range(2)] for (d0, half) in passes]
        for p in range(min(T2AHEAD, len(passes))):
            for (d, c) in t2jobs[p]:
                t2(d, c)
        for p, (d0, half) in enumerate(passes):
            if T2AHEAD > 0 and p + T2AHEAD < len(passes):
                for (d, c) in t2jobs[p + T2AHEAD]:
                    t2(d, c)
            stage_e(d0, half)

        with sc("w_g"):
            ct[2].wait()

        def revrows(z):
            nq = z.shape[0] // 8
            idx = 7 - jax.lax.broadcasted_iota(jnp.int32, (8, z.shape[1]), 0)
            return jnp.concatenate(
                [jnp.take_along_axis(z[8 * q:8 * q + 8], idx, axis=0) for q in range(nq - 1, -1, -1)], axis=0)

        def prep_a(i):
            Y = []
            for gam in range(NG):
                rs = pl.ds(8 * gam, 8)
                x = [(Sg(VI[0, i, d0, rs, :]), Sg(VI[1, i, d0, rs, :])) for d0 in range(4)]
                X = _dft4(x, +1)
                Y.append((jnp.concatenate([X[b1][0].val() for b1 in range(4)], axis=1),
                          jnp.concatenate([X[b1][1].val() for b1 in range(4)], axis=1)))
            zero = jnp.zeros((8, BM), f32)
            for blk in range(4):
                c, odd = blk % 2, blk // 2
                ng = 15 - odd
                for q in range(8):
                    rows = [Y[2 * g + odd][c] if g < ng else zero for g in (2 * q, 2 * q + 1)]
                    YB[i % 2, blk, pl.ds(16 * q, 16), :] = jnp.concatenate(rows, axis=0).astype(bf16)

        def prep_d(i, l0=0, l1=4):
            ls = slice(128 * l0, 128 * l1)
            Ce = jnp.dot(_asbf(GS[0]), YB[i % 2, 0, :, ls], preferred_element_type=f32)
            Se = jnp.dot(_asbf(GS[1]), YB[i % 2, 1, :, ls], preferred_element_type=f32)
            Co = jnp.dot(_asbf(GS[2]), YB[i % 2, 2, :, ls], preferred_element_type=f32)
            So = jnp.dot(_asbf(GS[3]), YB[i % 2, 3, :, ls], preferred_element_type=f32)
            return Ce, Se, Co, So

        def prep_b(i, z, l0=0, l1=4):
            Ce, Se, Co, So = z
            ls = slice(128 * l0, 128 * l1)
            pp = Ce + Co
            mm = Ce - Co
            qq = Se + So
            rr = So - Se
            y = jnp.concatenate([mm + rr, revrows(pp + qq), pp - qq, revrows(mm - rr)], axis=0)
            xw = jnp.concatenate([XS[i + 4 * b1] for b1 in range(l0, l1)], axis=1)
            h = (xw.astype(f32) + y).astype(bf16).astype(f32)
            mu = jnp.mean(h, axis=0, keepdims=True)
            hc = h - mu
            var = jnp.mean(hc * hc, axis=0, keepdims=True)
            a = (hc * jax.lax.rsqrt(var + EPS)).astype(bf16)
            AT[i, ls, :] = a.T
            ACC[i, :, ls] = h

        def mlp_up(i, j, l0=0, l1=4):
            sl = slice(j * FC, (j + 1) * FC)
            at = AT[i, 128 * l0:128 * l1, :]
            g = jnp.dot(at, WG[:, sl], preferred_element_type=f32)
            u = jnp.dot(at, WU[:, sl], preferred_element_type=f32)
            return (g * u).astype(bf16)

        def mlp_down(i, j, hh, l0=0, l1=4):
            sl = slice(j * FC, (j + 1) * FC)
            ls = slice(128 * l0, 128 * l1)
            acc = ACC[i, :, ls] + jax.lax.dot_general(WD[:, sl], hh, NTDIMS, preferred_element_type=f32)
            if j == NCH - 1:
                ob = acc.astype(bf16)
                for b1 in range(l0, l1):
                    OS[i + 4 * b1] = ob[:, 128 * (b1 - l0):128 * (b1 - l0) + 128]
                for b1 in range(l0, l1):
                    out_copy(i + 4 * b1).start()
            else:
                ACC[i, :, ls] = acc

        def do_mlp(i, j, l0=0, l1=4):
            mlp_down(i, j, mlp_up(i, j, l0, l1), l0, l1)

        def out_copy(t):
            off = t * 128 if isinstance(t, int) else pl.multiple_of(t * 128, 128)
            return pltpu.make_async_copy(OS.at[t], o_hbm.at[:, pl.ds(off, 128)], sem_o.at[0])

        prep_a(0)
        if SPLIT0:
            prep_b(0, prep_d(0, 0, 2), 0, 2)
        else:
            prep_b(0, prep_d(0))
        for j in range(NCH):
            with sc("w_m"):
                for c in cm[j]:
                    c.wait()
            if j + 1 < NCH:
                for c in cm[j + 1]:
                    c.start()
            if j == 0:
                for i in range(NB):
                    if i == 0 and SPLIT0:
                        z = prep_d(0, 2, 4)
                        hh = mlp_up(0, 0, 0, 2)
                        prep_b(0, z, 2, 4)
                        mlp_down(0, 0, hh, 0, 2)
                        prep_a(1)
                        hh = mlp_up(0, 0, 2, 4)
                        z = prep_d(1)
                        mlp_down(0, 0, hh, 2, 4)
                        prep_b(1, z)
                        continue
                    if i + 1 < NB:
                        prep_a(i + 1)
                    hh = mlp_up(i, 0)
                    if i + 1 < NB:
                        z = prep_d(i + 1)
                    mlp_down(i, 0, hh)
                    if i + 1 < NB:
                        prep_b(i + 1, z)
            elif P0MODE == "unroll":
                for i in range(NB):
                    do_mlp(i, j)
            else:
                nloop = NB - 1 if (SPLITL and j == NCH - 1) else NB

                def body(i, carry, j=j):
                    do_mlp(i, j)
                    return carry
                jax.lax.fori_loop(0, nloop, body, 0)
                if nloop < NB:
                    for (l0, l1) in SPLITL:
                        do_mlp(NB - 1, j, l0, l1)
        with sc("w_out"):
            for t in range(16):
                out_copy(t).wait()
    return _kernel


def build(interpret=False, FC=896, WWAITS=((2, 0, 8), (6, 8, 16)), WSTART=2, P0MODE="loop", T2AHEAD=1, XPRI=(0, 1, 1, 1), MGEN=1, MGEN0=3, SCOPES=False, EORDER=1, SPLIT0=True, SPLITL=(), fl=()):
    names = dict(lp='XLA_TPU_FORCE_LP_LLO_SCHEDULER', ev='XLA_TPU_EVENLY_DISTRIBUTE_CRITICAL_NODES', dd='XLA_TPU_RESCHEDULE_DMA_DONES', sl='XLA_TPU_ENABLE_LLO_SMALL_LOOP_FLATTENING')
    flags = {names[k]: True for k in fl} or None

    def fn(A_x, A_w_r, A_w_i, B_x, B_w_gate, B_w_up, B_w_down):
        Ft, G, base = _tables()
        xt = jnp.transpose(A_x, (0, 2, 1)).reshape(D, S)
        any_spec = pl.BlockSpec(memory_space=pl.ANY)
        R = 8 * NG
        out = pl.pallas_call(
            _make_kernel(FC, WWAITS, WSTART, P0MODE, T2AHEAD, XPRI, MGEN, MGEN0, SCOPES, EORDER, SPLIT0, SPLITL),
            out_shape=jax.ShapeDtypeStruct((D, S), bf16),
            in_specs=[any_spec] * 9,
            out_specs=any_spec,
            scratch_shapes=[
                pltpu.VMEM((16, D, 128), bf16),
                pltpu.VMEM((2, 16, K, 128), bf16),
                pltpu.VMEM((2, 16, 8 * WPITCH, 128), f32),
                pltpu.VMEM((2, 16, 120, 128), f32),
                pltpu.VMEM((2, 4, 4, R, 128), f32),
                pltpu.VMEM((2, 16, R, 128), f32),
                pltpu.VMEM((2, 2, R, 128), f32),
                pltpu.VMEM((4, 2, 2, R, 128), f32),
                pltpu.VMEM((2, 4, 4, R, 128), f32),
                pltpu.VMEM((2, 4, 128, BM), bf16),
                pltpu.VMEM((4, 64, 128), u32),
                pltpu.VMEM((4, 56, 128), u32),
                pltpu.VMEM((288, 128), f32),
                pltpu.VMEM((16, 2, 128, 128), bf16),
                pltpu.VMEM((D, F), bf16),
                pltpu.VMEM((D, F), bf16),
                pltpu.VMEM((D, F), bf16),
                pltpu.VMEM((16, D, 128), bf16),
                pltpu.VMEM((NB, BM, D), bf16),
                pltpu.VMEM((NB, D, BM), f32),
                pltpu.SemaphoreType.DMA((4,)),
                pltpu.SemaphoreType.DMA((len(WWAITS),)),
                pltpu.SemaphoreType.DMA((2,)),
                pltpu.SemaphoreType.DMA((F // FC,)),
                pltpu.SemaphoreType.DMA((1,)),
            ],
            compiler_params=pltpu.CompilerParams(vmem_limit_bytes=100 * 2**20, flags=flags),
            interpret=(pltpu.InterpretParams() if interpret else False),
        )(xt, A_w_r.T, A_w_i.T, B_w_gate, B_w_up, B_w_down.T, jnp.asarray(Ft), jnp.asarray(G), jnp.asarray(base))
        return jnp.transpose(out.reshape(1, D, S), (0, 2, 1))
    return jax.jit(fn)


_forward = build()


@jax.jit
def pallas_sequential_preLN__spectral_gfnet__glu_gated_bilinear__prompt_kernel(
    A_x: jax.Array,
    A_w_r: jax.Array,
    A_w_i: jax.Array,
    B_x: jax.Array,
    B_w_gate: jax.Array,
    B_w_up: jax.Array,
    B_w_down: jax.Array,
):
    return _forward(A_x, A_w_r, A_w_i, B_x, B_w_gate, B_w_up, B_w_down)
```

```python
import numpy as np
import jax
import jax.numpy as jnp
import jax.experimental.pallas as pl
import jax.experimental.pallas.tpu as pltpu

S, D, F, K = 2048, 448, 1792, 225
EPS = 1e-5
bf16, f32, u32 = jnp.bfloat16, jnp.float32, jnp.uint32
NTDIMS = (((1,), (1,)), ((), ()))
NG = 29
WPITCH = 17
NB = 4
BM = S // NB


def _pack_rows(a):
    import ml_dtypes
    b = a.astype(ml_dtypes.bfloat16).view(np.uint16).astype(np.uint32)
    return b[..., 0::2, :] | (b[..., 1::2, :] << 16)


def _tables():
    th = 2 * np.pi / D
    nu = np.arange(112) + 0.5
    n = []
    for v in range(7):
        n += [16 * v + 2 * i for i in range(8)] + [16 * v + 2 * i + 1 for i in range(8)]
    nuf = np.array(n) + 0.5
    kE = 2 * np.arange(113)
    kO = 2 * np.arange(112) + 1
    Ft = np.zeros((4, 128, 128))
    Ft[0, :113, :112] = np.cos(np.outer(kE, nuf) * th)
    Ft[0, 112, :] = 0
    Ft[1, :113, :112] = -np.sin(np.outer(kE, nuf) * th)
    Ft[1, 0, :] = 0
    Ft[2, :112, :112] = np.cos(np.outer(kO, nuf) * th)
    Ft[3, :112, :112] = -np.sin(np.outer(kO, nuf) * th)
    cE = np.full(113, 2.0)
    cE[0] = 1
    cE[112] = 1
    sc = 1.0 / (D * S)
    G = np.zeros((4, 112, 128))
    gce = np.cos(np.outer(nu, kE) * th)
    gce[:, 112] = 0
    gse = np.sin(np.outer(nu, kE) * th)
    gse[:, 0] = 0
    G[0, :, :113] = gce * cE * sc
    G[1, :, :113] = gse * cE * sc
    G[2, :, :112] = np.cos(np.outer(nu, kO) * th) * 2 * sc
    G[3, :, :112] = np.sin(np.outer(nu, kO) * th) * 2 * sc
    a = np.arange(128)
    base = np.zeros((80, 128), np.float32)
    pg = -2 * np.pi * (np.outer(np.arange(8), a) % 128) / 128
    pu = -2 * np.pi * (np.outer(8 * np.arange(16), a) % 128) / 128
    pt = -2 * np.pi * np.outer(np.arange(16), a) / S
    base[0:8], base[8:16] = np.cos(pg), np.sin(pg)
    base[16:32], base[32:48] = np.cos(pu), np.sin(pu)
    base[48:64], base[64:80] = np.cos(pt), np.sin(pt)
    return _pack_rows(Ft), _pack_rows(G), base


class Sg:
    __slots__ = ("v", "s")

    def __init__(self, v, s=1):
        self.v, self.s = v, s

    def __neg__(self):
        return Sg(self.v, -self.s)

    def __add__(self, o):
        if self.s == o.s:
            return Sg(self.v + o.v, self.s)
        if self.s > 0:
            return Sg(self.v - o.v, 1)
        return Sg(o.v - self.v, 1)

    def __sub__(self, o):
        return self + (-o)

    def scale(self, c):
        return Sg(self.v * np.float32(c * self.s), 1)

    def val(self):
        return self.v if self.s > 0 else -self.v


def _dft4_finish(t0, t1, t2, t3, sgn):
    X0 = (t0[0] + t2[0], t0[1] + t2[1])
    X2 = (t0[0] - t2[0], t0[1] - t2[1])
    XA = (t1[0] + t3[1], t1[1] - t3[0])
    XB = (t1[0] - t3[1], t1[1] + t3[0])
    if sgn < 0:
        return [X0, XA, X2, XB]
    return [X0, XB, X2, XA]


def _dft4(x, sgn):
    (r0, i0), (r1, i1), (r2, i2), (r3, i3) = x
    return _dft4_finish((r0 + r2, i0 + i2), (r0 - r2, i0 - i2), (r1 + r3, i1 + i3), (r1 - r3, i1 - i3), sgn)


def _dft4_one(x, k, sgn):
    if k % 2 == 0:
        t0 = (x[0][0] + x[2][0], x[0][1] + x[2][1])
        t2 = (x[1][0] + x[3][0], x[1][1] + x[3][1])
        return (t0[0] + t2[0], t0[1] + t2[1]) if k == 0 else (t0[0] - t2[0], t0[1] - t2[1])
    t1 = (x[0][0] - x[2][0], x[0][1] - x[2][1])
    t3 = (x[1][0] - x[3][0], x[1][1] - x[3][1])
    if (k == 1) == (sgn < 0):
        return (t1[0] + t3[1], t1[1] - t3[0])
    return (t1[0] - t3[1], t1[1] + t3[0])


def _dft4_two(x, par, sgn):
    if par == 0:
        t0 = (x[0][0] + x[2][0], x[0][1] + x[2][1])
        t2 = (x[1][0] + x[3][0], x[1][1] + x[3][1])
        return [(t0[0] + t2[0], t0[1] + t2[1]), (t0[0] - t2[0], t0[1] - t2[1])]
    t1 = (x[0][0] - x[2][0], x[0][1] - x[2][1])
    t3 = (x[1][0] - x[3][0], x[1][1] - x[3][1])
    xa = (t1[0] + t3[1], t1[1] - t3[0])
    xb = (t1[0] - t3[1], t1[1] + t3[0])
    return [xa, xb] if sgn < 0 else [xb, xa]


def _tw16(z, e, sgn):
    r, i = z
    e = e % 16
    if e == 0:
        return z
    if e == 4:
        return (i, -r) if sgn < 0 else (-i, r)
    if e == 8:
        return (-r, -i)
    if e == 12:
        return (-i, r) if sgn < 0 else (i, -r)
    h = float(np.sqrt(0.5))
    if e in (2, 6, 10, 14):
        c = h if e in (2, 14) else -h
        s = h * sgn * (1 if e < 8 else -1)
        re = (r if c > 0 else -r) - (i if s > 0 else -i)
        im = (r if s > 0 else -r) + (i if c > 0 else -i)
        return (re.scale(h), im.scale(h))
    c = float(np.cos(2 * np.pi * e / 16))
    s = float(sgn * np.sin(2 * np.pi * e / 16))
    return (r.scale(c) - i.scale(s), r.scale(s) + i.scale(c))


def _sg(z):
    return (Sg(z[0]), Sg(z[1]))


def _bf_lo(u):
    return pltpu.bitcast(u << 16, f32)


def _bf_hi(u):
    return pltpu.bitcast(u & np.uint32(0xFFFF0000), f32)


def _asbf(u):
    return pltpu.bitcast(u, bf16)


import contextlib


def _make_kernel(FC, WWAITS, WSTART, P0MODE, T2AHEAD, XPRI, XG, FPRI, SCOPES, SPLIT0, SPLITL, OPQ, CM, EM, ANN, MG, THR, OPW):
    def sc(name):
        return jax.named_scope(name) if SCOPES else contextlib.nullcontext()

    NCH = F // FC

    def _kernel(x_hbm, wr_hbm, wi_hbm, wg_hbm, wu_hbm, wd_hbm, f_hbm, g_hbm, b_hbm, o_hbm,
                XS, WS, BUF, WP, VF, FP, YB, FS, GS, BS, MS, WG, WU, WD, OS, AT, ACC,
                zi_ref, sem_x, sem_w, sem_t, sem_m, sem_o):
        wgrp = {t: gi for gi, (_, a, b) in enumerate(WWAITS) for t in range(a, b)}
        xgrp = {j: gi for gi, pairs in enumerate(XG) for j in pairs}
        ct = [pltpu.make_async_copy(b_hbm, BS, sem_t.at[0]),
              pltpu.make_async_copy(f_hbm, FS, sem_t.at[1]),
              pltpu.make_async_copy(g_hbm, GS, sem_t.at[2])]
        cx = [pltpu.make_async_copy(x_hbm.at[:, pl.ds(t * 128, 128)], XS.at[t], sem_x.at[xgrp[t % 8]]) for t in range(16)]
        cw = [[pltpu.make_async_copy(w.at[:, pl.ds(t * 128, 128)], WS.at[c, t], sem_w.at[wgrp[t]]) for t in range(16)]
              for c, w in enumerate((wr_hbm, wi_hbm))]
        cm = [[pltpu.make_async_copy(a.at[:, pl.ds(j * FC, FC)], b.at[:, pl.ds(j * FC, FC)], sem_m.at[j])
               for i, (a, b) in enumerate(((wg_hbm, WG), (wu_hbm, WU), (wd_hbm, WD)))] for j in range(NCH)]
        if not MG:
            ct[0].start(priority=0)
        ct[1].start(priority=FPRI)
        for gi, pairs in enumerate(XG):
            for j in pairs:
                cx[j].start(priority=XPRI[gi])
                cx[j + 8].start(priority=XPRI[gi])
        if MG:
            ct[0].start(priority=1)

        if ANN:
            XS, WS, FS, GS, BS, WG, WU, WD = [pltpu.annotate(r, no_store=True) for r in (XS, WS, FS, GS, BS, WG, WU, WD)]
        row8 = jax.lax.broadcasted_iota(jnp.int32, (8, 128), 0)
        rev8 = 7 - row8

        def _zero(i, carry):
            zi_ref[i] = 0
            return carry
        jax.lax.fori_loop(0, 16, _zero, 0)

        def gen_m(d):
            gr, gi_ = BS[0:8, :], BS[8:16, :]
            ur, ui = BS[16:32, :], BS[32:48, :]
            if d == 0:
                c_r, c_i = ur, ui
            else:
                twr = jnp.broadcast_to(BS[48 + d:49 + d, :], (16, 128))
                twi = jnp.broadcast_to(BS[64 + d:65 + d, :], (16, 128))
                c_r = ur * twr - ui * twi
                c_i = ur * twi + ui * twr
            for q2 in range(8):
                m0, m1, m2, m3 = [], [], [], []
                for q in (2 * q2, 2 * q2 + 1):
                    cr = jnp.broadcast_to(c_r[q:q + 1, :], (8, 128))
                    ci = jnp.broadcast_to(c_i[q:q + 1, :], (8, 128))
                    mr = gr * cr - gi_ * ci
                    mi = gr * ci + gi_ * cr
                    m0.append(mr)
                    m1.append(mr + mi)
                    m2.append(mr - mi)
                    m3.append(mi)
                for k_, m in enumerate((m0, m1, m2, m3)):
                    if (k_ in (1, 2) and 3 not in (CM, EM)) or (k_ == 3 and 4 not in (CM, EM)):
                        continue
                    MS[d, k_, pl.ds(16 * q2, 16), :] = jnp.concatenate(m, axis=0).astype(bf16)

        if MG == 0:
            with sc("w_tab"):
                ct[0].wait()
            for d in range(16):
                gen_m(d)
        with sc("w_f"):
            ct[1].wait()

        def fold_tile(t):
            def ld(v, reverse):
                u = pltpu.bitcast(XS[t, pl.ds(16 * v, 16), :], u32)
                if reverse:
                    u = jnp.take_along_axis(u, rev8, axis=0)
                return _bf_lo(u), _bf_hi(u)
            Ree, Ro, Ie, Io = [], [], [], []
            sq = None
            for v in range(7):
                Al, Ah = ld(v, False)
                Bl, Bh = ld(27 - v, True)
                Cl, Ch = ld(13 - v, True)
                Dl, Dh = ld(14 + v, False)
                for (a, b, c, d) in ((Al, Bh, Ch, Dl), (Ah, Bl, Cl, Dh)):
                    p = a + b
                    q = c + d
                    r = a - b
                    s = d - c
                    ro, ie, io = q - p, s + r, s - r
                    Ree.append(q + p)
                    Ro.append(ro)
                    Ie.append(ie)
                    Io.append(io)
                    t2 = ro * ro + ie * ie + io * io
                    sq = t2 if sq is None else sq + t2
            tot = Ree[0]
            for z in Ree[1:]:
                tot = tot + z
            mean4 = jnp.sum(tot, axis=0, keepdims=True) * np.float32(4.0 / D)
            Ree = [z - mean4 for z in Ree]
            for z in Ree:
                sq = sq + z * z
            var = jnp.sum(sq, axis=0, keepdims=True) * np.float32(1.0 / (4 * D))
            rstd = jax.lax.rsqrt(var + EPS)
            return (Ree, Ie, Ro, Io), rstd

        def stage_a(j):
            parts = [fold_tile(j), fold_tile(j + 8)]
            rstd = jnp.concatenate([p[1] for p in parts], axis=1)
            zpad = jnp.zeros((16, 256), f32)
            for odd in (1, 0):
                z = []
                for blk in (2 * odd, 2 * odd + 1):
                    rows = [jnp.concatenate([parts[i][0][blk][v] for i in range(2)], axis=1) for v in range(14)]
                    data = jnp.concatenate(rows + [zpad], axis=0).astype(bf16)
                    nrow = 56 if odd else 64
                    z.append(jnp.dot(_asbf(FS[blk, 0:nrow, :]), data, preferred_element_type=f32))
                for g in range(15 - odd):
                    rs = pl.ds(16 * g + 8 * odd, 8)
                    zr = z[0][8 * g:8 * g + 8, :] * rstd
                    zi = z[1][8 * g:8 * g + 8, :] * rstd
                    xa = (Sg(zr[:, 0:128]), Sg(zi[:, 0:128]))
                    xb = (Sg(zr[:, 128:256]), Sg(zi[:, 128:256]))
                    sm = (xa[0] + xb[0], xa[1] + xb[1])
                    df = _tw16((xa[0] - xb[0], xa[1] - xb[1]), j, -1)
                    VF[0, 0, j, rs, :] = sm[0].val()
                    VF[1, 0, j, rs, :] = sm[1].val()
                    VF[0, 1, j, rs, :] = df[0].val()
                    VF[1, 1, j, rs, :] = df[1].val()

        for gi, pairs in enumerate(XG):
            with sc("w_x"):
                for j in pairs:
                    cx[j].wait()
                    cx[j + 8].wait()
            if gi == WSTART:
                for t in range(16):
                    cw[0][t].start(priority=1)
                    cw[1][t].start(priority=1)
            if gi == len(XG) - 1:
                ct[2].start(priority=1)
                for c in cm[0]:
                    c.start(priority=1)
            for j in pairs:
                stage_a(j)
            if MG and gi == len(XG) - 1:
                with sc("w_tab"):
                    ct[0].wait()
                gen_m(0)
                gen_m(8)

        NWT = 2 * 16 * 8 * WPITCH

        def wt_row(c, t, z=0):
            return (c * 16 + t) * 8 * WPITCH + z

        def vi_rows(c, par, d, gam, z=0):
            r = NWT + ((c * 2 + par) * 8 + d) * 8 * NG + 8 * gam + z
            return pl.ds(r if isinstance(r, int) else pl.multiple_of(r, 8), 8)

        def t1(t, c):
            u = pltpu.bitcast(WS[c, t, 0:224, :], u32)
            w224 = pltpu.bitcast(WS[c, t, 224:225, :].astype(f32), u32) >> 16
            last = jnp.where(row8 == 0, jnp.broadcast_to(w224, (8, 128)), np.uint32(0))
            full = jnp.concatenate([u, last, jnp.zeros((8, 128), u32)], axis=0)
            ut = pltpu.bitcast(full, f32).T
            for q in range(8):
                BUF[pl.ds(wt_row(c, t) + WPITCH * q, 16), :] = ut[16 * q:16 * q + 16, :]

        def t2(d, c):
            z = zi_ref[d % 8] if THR else 0
            Gm = jnp.concatenate([BUF[pl.ds(wt_row(c, t, z) + d, 8, stride=WPITCH), :] for t in range(16)], axis=0)
            WP[c, d] = Gm.T[0:120, :]

        def three_dots(zr, zi, d, nt):
            pad = [jnp.zeros((8, 128), f32)]
            ls = [jnp.concatenate([a_ + b_ for a_, b_ in zip(zr, zi)] + pad, axis=0).astype(bf16),
                  jnp.concatenate(zi + pad, axis=0).astype(bf16),
                  jnp.concatenate(zr + pad, axis=0).astype(bf16)]
            if nt:
                ms = (MS[d, 0], MS[d, 1], MS[d, 2])
                k = [jax.lax.dot_general(l, m, NTDIMS, preferred_element_type=f32) for l, m in zip(ls, ms)]
            else:
                ms = (MS[d, 0], MS[d, 2], MS[d, 1])
                k = [jnp.dot(l, m, preferred_element_type=f32) for l, m in zip(ls, ms)]
            out = []
            for gam in range(NG):
                r = slice(8 * gam, 8 * gam + 8)
                out.append((k[0][r] - k[1][r], k[0][r] - k[2][r]))
            return out

        def four_dots(zr, zi, d, nt):
            rows = []
            for a_, b_ in zip(zr, zi):
                rows += [a_, b_]
            lhs = jnp.concatenate(rows, axis=0).astype(bf16)
            if nt:
                A = jax.lax.dot_general(lhs, MS[d, 0], NTDIMS, preferred_element_type=f32)
                B = jax.lax.dot_general(lhs, MS[d, 3], NTDIMS, preferred_element_type=f32)
            else:
                A = jnp.dot(lhs, MS[d, 0], preferred_element_type=f32)
                B = jnp.dot(lhs, MS[d, 3], preferred_element_type=f32)
            out = []
            for gam in range(NG):
                r = 16 * gam
                if nt:
                    out.append((A[r:r + 8] - B[r + 8:r + 16], B[r:r + 8] + A[r + 8:r + 16]))
                else:
                    out.append((A[r:r + 8] + B[r + 8:r + 16], A[r + 8:r + 16] - B[r:r + 8]))
            return out

        def stage_c(d):
            par, dp = d % 2 + (zi_ref[d] if OPQ else 0), d // 2
            ar, ai, br, bi = [], [], [], []
            for gam in range(NG):
                rs = pl.ds(8 * gam, 8)
                v = [(Sg(VF[0, par, j, rs, :]), Sg(VF[1, par, j, rs, :])) for j in range(8)]
                e4 = _dft4_one([v[0], v[2], v[4], v[6]], dp, -1)
                o4 = _tw16(_dft4_one([v[1], v[3], v[5], v[7]], dp, -1), 2 * dp, -1)
                ar.append((e4[0] + o4[0]).val())
                ai.append((e4[1] + o4[1]).val())
                br.append((e4[0] - o4[0]).val())
                bi.append((e4[1] - o4[1]).val())
            for dd, zr, zi in ((d, ar, ai), (d + 8, br, bi)):
                out = (three_dots if CM == 3 else four_dots)(zr, zi, dd, True)
                for gam in range(NG):
                    FP[0, dd, pl.ds(8 * gam, 8), :] = out[gam][0]
                    FP[1, dd, pl.ds(8 * gam, 8), :] = out[gam][1]

        passes = list(range(8))
        wwait = {p: (a, b) for (p, a, b) in WWAITS}
        pending, per = [], 0
        for p in passes:
            if p in wwait:
                a, b = wwait[p]
                with sc("w_w"):
                    for t in range(a, b):
                        cw[0][t].wait()
                        cw[1][t].wait()
                pending = [(t, c) for t in range(a, b) for c in range(2)]
                nxt = [q for q in sorted(wwait) if q > p]
                span = (nxt[0] if nxt else len(passes)) - p
                per = -(-len(pending) // span)
            for (t, c) in pending[:per]:
                t1(t, c)
            pending = pending[per:]
            if MG and p + 1 < 8:
                gen_m(p + 1)
                gen_m(p + 9)
            stage_c(p)
        assert not pending

        def w_mul(d):
            pr, pi = [], []
            for gam in range(NG):
                gg, odd = gam // 2, gam % 2
                wu_r = pltpu.bitcast(WP[0, d, pl.ds(8 * gg, 8), :], u32)
                wu_i = pltpu.bitcast(WP[1, d, pl.ds(8 * gg, 8), :], u32)
                wr_ = _bf_hi(wu_r) if odd else _bf_lo(wu_r)
                wi_ = _bf_hi(wu_i) if odd else _bf_lo(wu_i)
                zr = FP[0, d, pl.ds(8 * gam, 8), :]
                zi = FP[1, d, pl.ds(8 * gam, 8), :]
                pr.append(zr * wr_ - zi * wi_)
                pi.append(zr * wi_ + zi * wr_)
            return (three_dots if EM == 3 else four_dots)(pr, pi, d, False)

        def stage_e(d):
            ua = w_mul(d)
            ub = w_mul(d + 8)
            for gam in range(NG):
                rs = pl.ds(8 * gam, 8)
                xa, xb = _sg(ua[gam]), _sg(ub[gam])
                sm = (xa[0] + xb[0], xa[1] + xb[1])
                df = _tw16((xa[0] - xb[0], xa[1] - xb[1]), d, +1)
                z = zi_ref[8 + d] if THR else 0
                BUF[vi_rows(0, 0, d, gam, z), :] = sm[0].val()
                BUF[vi_rows(1, 0, d, gam, z), :] = sm[1].val()
                BUF[vi_rows(0, 1, d, gam, z), :] = df[0].val()
                BUF[vi_rows(1, 1, d, gam, z), :] = df[1].val()

        t2jobs = [[(d + 8 * s_, c) for s_ in range(2) for c in range(2)] for d in range(8)]
        for p in range(T2AHEAD):
            for (d, c) in t2jobs[p]:
                t2(d, c)
        for p in range(8):
            if not THR and p + T2AHEAD < 8:
                for (d, c) in t2jobs[p + T2AHEAD]:
                    t2(d, c)
            stage_e(p)
            if THR and p + T2AHEAD < 8:
                for (d, c) in t2jobs[p + T2AHEAD]:
                    t2(d, c)

        with sc("w_g"):
            ct[2].wait()

        def revrows(z):
            nq = z.shape[0] // 8
            idx = 7 - jax.lax.broadcasted_iota(jnp.int32, (8, z.shape[1]), 0)
            return jnp.concatenate(
                [jnp.take_along_axis(z[8 * q:8 * q + 8], idx, axis=0) for q in range(nq - 1, -1, -1)], axis=0)

        def prep_a(i):
            par, typ = i % 2, i // 2
            zz = zi_ref[8 + i] if OPQ else 0
            Y = []
            for gam in range(NG):
                rs = pl.ds(8 * gam, 8)
                w = [(Sg(BUF[vi_rows(0, par, d, gam, zz), :]), Sg(BUF[vi_rows(1, par, d, gam, zz), :])) for d in range(8)]
                ev = _dft4_two([w[0], w[2], w[4], w[6]], typ, +1)
                od = _dft4_two([w[1], w[3], w[5], w[7]], typ, +1)
                outs = {}
                for kk, bp in enumerate((typ, typ + 2)):
                    o4 = _tw16(od[kk], 2 * bp, +1)
                    outs[bp] = (ev[kk][0] + o4[0], ev[kk][1] + o4[1])
                    outs[bp + 4] = (ev[kk][0] - o4[0], ev[kk][1] - o4[1])
                X = [outs[typ + 2 * b1] for b1 in range(4)]
                Y.append((jnp.concatenate([X[b1][0].val() for b1 in range(4)], axis=1),
                          jnp.concatenate([X[b1][1].val() for b1 in range(4)], axis=1)))
            zero = jnp.zeros((8, BM), f32)
            for blk in range(4):
                c, odd = blk % 2, blk // 2
                ng = 15 - odd
                for q in range(8):
                    rows = [Y[2 * g + odd][c] if g < ng else zero for g in (2 * q, 2 * q + 1)]
                    YB[i % 2, blk, pl.ds(16 * q, 16), :] = jnp.concatenate(rows, axis=0).astype(bf16)

        def prep_d(i, l0=0, l1=4):
            ls = slice(128 * l0, 128 * l1)
            Ce = jnp.dot(_asbf(GS[0]), YB[i % 2, 0, :, ls], preferred_element_type=f32)
            Se = jnp.dot(_asbf(GS[1]), YB[i % 2, 1, :, ls], preferred_element_type=f32)
            Co = jnp.dot(_asbf(GS[2]), YB[i % 2, 2, :, ls], preferred_element_type=f32)
            So = jnp.dot(_asbf(GS[3]), YB[i % 2, 3, :, ls], preferred_element_type=f32)
            return Ce, Se, Co, So

        def prep_b(i, z, l0=0, l1=4):
            Ce, Se, Co, So = z
            ls = slice(128 * l0, 128 * l1)
            pp = Ce + Co
            mm = Ce - Co
            qq = Se + So
            rr = So - Se
            y = jnp.concatenate([mm + rr, revrows(pp + qq), pp - qq, revrows(mm - rr)], axis=0)
            xw = jnp.concatenate([XS[i + 4 * b1] for b1 in range(l0, l1)], axis=1)
            h = (xw.astype(f32) + y).astype(bf16).astype(f32)
            mu = jnp.mean(h, axis=0, keepdims=True)
            hc = h - mu
            var = jnp.mean(hc * hc, axis=0, keepdims=True)
            a = (hc * jax.lax.rsqrt(var + EPS)).astype(bf16)
            AT[i, ls, :] = a.T
            ACC[i, :, ls] = h

        def fslice(i, j):
            if OPW and isinstance(i, int):
                return pl.ds(pl.multiple_of(j * FC + zi_ref[12 + i], 128), FC)
            return slice(j * FC, (j + 1) * FC)

        def mlp_up(i, j, l0=0, l1=4):
            sl = fslice(i, j)
            at = AT[i, 128 * l0:128 * l1, :]
            g = jnp.dot(at, WG[:, sl], preferred_element_type=f32)
            u = jnp.dot(at, WU[:, sl], preferred_element_type=f32)
            return (g * u).astype(bf16)

        def mlp_down(i, j, hh, l0=0, l1=4):
            sl = fslice(i, j)
            ls = slice(128 * l0, 128 * l1)
            acc = ACC[i, :, ls] + jax.lax.dot_general(WD[:, sl], hh, NTDIMS, preferred_element_type=f32)
            if j == NCH - 1:
                ob = acc.astype(bf16)
                for b1 in range(l0, l1):
                    OS[i + 4 * b1] = ob[:, 128 * (b1 - l0):128 * (b1 - l0) + 128]
                for b1 in range(l0, l1):
                    out_copy(i + 4 * b1).start()
            else:
                ACC[i, :, ls] = acc

        def do_mlp(i, j, l0=0, l1=4):
            mlp_down(i, j, mlp_up(i, j, l0, l1), l0, l1)

        def out_copy(t):
            off = t * 128 if isinstance(t, int) else pl.multiple_of(t * 128, 128)
            return pltpu.make_async_copy(OS.at[t], o_hbm.at[:, pl.ds(off, 128)], sem_o.at[0])

        prep_a(0)
        if SPLIT0:
            prep_b(0, prep_d(0, 0, 2), 0, 2)
        else:
            prep_b(0, prep_d(0))
        for j in range(NCH):
            with sc("w_m"):
                for c in cm[j]:
                    c.wait()
            if j + 1 < NCH:
                for c in cm[j + 1]:
                    c.start()
            if j == 0:
                for i in range(NB):
                    if i == 0 and SPLIT0:
                        z = prep_d(0, 2, 4)
                        hh = mlp_up(0, 0, 0, 2)
                        prep_b(0, z, 2, 4)
                        mlp_down(0, 0, hh, 0, 2)
                        prep_a(1)
                        hh = mlp_up(0, 0, 2, 4)
                        z = prep_d(1)
                        mlp_down(0, 0, hh, 2, 4)
                        prep_b(1, z)
                        continue
                    if i + 1 < NB:
                        prep_a(i + 1)
                    hh = mlp_up(i, 0)
                    if i + 1 < NB:
                        z = prep_d(i + 1)
                    mlp_down(i, 0, hh)
                    if i + 1 < NB:
                        prep_b(i + 1, z)
            elif P0MODE == "unroll":
                for i in range(NB):
                    do_mlp(i, j)
            else:
                nloop = NB - 1 if (SPLITL and j == NCH - 1) else NB

                def body(i, carry, j=j):
                    do_mlp(i, j)
                    return carry
                jax.lax.fori_loop(0, nloop, body, 0)
                if nloop < NB:
                    for (l0, l1) in SPLITL:
                        do_mlp(NB - 1, j, l0, l1)
        with sc("w_out"):
            for t in range(16):
                out_copy(t).wait()
    return _kernel


def build(interpret=False, FC=896, WWAITS=((2, 0, 8), (6, 8, 16)), WSTART=2, P0MODE="loop", T2AHEAD=1, XPRI=(1, 1, 1, 1), XG=((0, 1), (2, 3), (4, 5), (6, 7)), FPRI=0, SCOPES=False, SPLIT0=True, SPLITL=(), OPQ=True, CM=3, EM=3, ANN=False, MG=0, THR=False, OPW=False, fl=()):
    names = dict(lp='XLA_TPU_FORCE_LP_LLO_SCHEDULER', ev='XLA_TPU_EVENLY_DISTRIBUTE_CRITICAL_NODES', dd='XLA_TPU_RESCHEDULE_DMA_DONES', sl='XLA_TPU_ENABLE_LLO_SMALL_LOOP_FLATTENING')
    flags = {names[k]: True for k in fl} or None

    def fn(A_x, A_w_r, A_w_i, B_x, B_w_gate, B_w_up, B_w_down):
        Ft, G, base = _tables()
        xt = jnp.transpose(A_x, (0, 2, 1)).reshape(D, S)
        any_spec = pl.BlockSpec(memory_space=pl.ANY)
        R = 8 * NG
        out = pl.pallas_call(
            _make_kernel(FC, WWAITS, WSTART, P0MODE, T2AHEAD, XPRI, XG, FPRI, SCOPES, SPLIT0, SPLITL, OPQ, CM, EM, ANN, MG, THR, OPW),
            out_shape=jax.ShapeDtypeStruct((D, S), bf16),
            in_specs=[any_spec] * 9,
            out_specs=any_spec,
            scratch_shapes=[
                pltpu.VMEM((16, D, 128), bf16),
                pltpu.VMEM((2, 16, K, 128), bf16),
                pltpu.VMEM((2 * 16 * 8 * WPITCH + 32 * R, 128), f32),
                pltpu.VMEM((2, 16, 120, 128), f32),
                pltpu.VMEM((2, 2, 8, R, 128), f32),
                pltpu.VMEM((2, 16, R, 128), f32),
                pltpu.VMEM((2, 4, 128, BM), bf16),
                pltpu.VMEM((4, 64, 128), u32),
                pltpu.VMEM((4, 56, 128), u32),
                pltpu.VMEM((80, 128), f32),
                pltpu.VMEM((16, 4, 128, 128), bf16),
                pltpu.VMEM((D, F), bf16),
                pltpu.VMEM((D, F), bf16),
                pltpu.VMEM((D, F), bf16),
                pltpu.VMEM((16, D, 128), bf16),
                pltpu.VMEM((NB, BM, D), bf16),
                pltpu.VMEM((NB, D, BM), f32),
                pltpu.SMEM((16,), jnp.int32),
                pltpu.SemaphoreType.DMA((len(XG),)),
                pltpu.SemaphoreType.DMA((len(WWAITS),)),
                pltpu.SemaphoreType.DMA((3,)),
                pltpu.SemaphoreType.DMA((F // FC,)),
                pltpu.SemaphoreType.DMA((1,)),
            ],
            compiler_params=pltpu.CompilerParams(vmem_limit_bytes=100 * 2**20, flags=flags),
            interpret=(pltpu.InterpretParams() if interpret else False),
        )(xt, A_w_r.T, A_w_i.T, B_w_gate, B_w_up, B_w_down.T, jnp.asarray(Ft), jnp.asarray(G), jnp.asarray(base))
        return jnp.transpose(out.reshape(1, D, S), (0, 2, 1))
    return jax.jit(fn)


_forward = build()


@jax.jit
def pallas_sequential_preLN__spectral_gfnet__glu_gated_bilinear__prompt_kernel(
    A_x: jax.Array,
    A_w_r: jax.Array,
    A_w_i: jax.Array,
    B_x: jax.Array,
    B_w_gate: jax.Array,
    B_w_up: jax.Array,
    B_w_down: jax.Array,
):
    return _forward(A_x, A_w_r, A_w_i, B_x, B_w_gate, B_w_up, B_w_down)
```

```python
import numpy as np
import jax
import jax.numpy as jnp
import jax.experimental.pallas as pl
import jax.experimental.pallas.tpu as pltpu

S, D, F, K = 2048, 448, 1792, 225
EPS = 1e-5
bf16, f32, u32 = jnp.bfloat16, jnp.float32, jnp.uint32
NTDIMS = (((1,), (1,)), ((), ()))
NG = 29
WPITCH = 17
NB = 4
BM = S // NB


def _pack_rows(a):
    import ml_dtypes
    b = a.astype(ml_dtypes.bfloat16).view(np.uint16).astype(np.uint32)
    return b[..., 0::2, :] | (b[..., 1::2, :] << 16)


def _tables():
    th = 2 * np.pi / D
    nu = np.arange(112) + 0.5
    n = []
    for v in range(7):
        n += [16 * v + 2 * i for i in range(8)] + [16 * v + 2 * i + 1 for i in range(8)]
    nuf = np.array(n) + 0.5
    kE = 2 * np.arange(113)
    kO = 2 * np.arange(112) + 1
    Ft = np.zeros((4, 128, 128))
    Ft[0, :113, :112] = np.cos(np.outer(kE, nuf) * th)
    Ft[0, 112, :] = 0
    Ft[1, :113, :112] = -np.sin(np.outer(kE, nuf) * th)
    Ft[1, 0, :] = 0
    Ft[2, :112, :112] = np.cos(np.outer(kO, nuf) * th)
    Ft[3, :112, :112] = -np.sin(np.outer(kO, nuf) * th)
    cE = np.full(113, 2.0)
    cE[0] = 1
    cE[112] = 1
    sc = 1.0 / (D * S)
    G = np.zeros((4, 112, 128))
    gce = np.cos(np.outer(nu, kE) * th)
    gce[:, 112] = 0
    gse = np.sin(np.outer(nu, kE) * th)
    gse[:, 0] = 0
    G[0, :, :113] = gce * cE * sc
    G[1, :, :113] = gse * cE * sc
    G[2, :, :112] = np.cos(np.outer(nu, kO) * th) * 2 * sc
    G[3, :, :112] = np.sin(np.outer(nu, kO) * th) * 2 * sc
    a = np.arange(128)
    base = np.zeros((80, 128), np.float32)
    pg = -2 * np.pi * (np.outer(np.arange(8), a) % 128) / 128
    pu = -2 * np.pi * (np.outer(8 * np.arange(16), a) % 128) / 128
    pt = -2 * np.pi * np.outer(np.arange(16), a) / S
    base[0:8], base[8:16] = np.cos(pg), np.sin(pg)
    base[16:32], base[32:48] = np.cos(pu), np.sin(pu)
    base[48:64], base[64:80] = np.cos(pt), np.sin(pt)
    return _pack_rows(Ft), _pack_rows(G), base


class Sg:
    __slots__ = ("v", "s")

    def __init__(self, v, s=1):
        self.v, self.s = v, s

    def __neg__(self):
        return Sg(self.v, -self.s)

    def __add__(self, o):
        if self.s == o.s:
            return Sg(self.v + o.v, self.s)
        if self.s > 0:
            return Sg(self.v - o.v, 1)
        return Sg(o.v - self.v, 1)

    def __sub__(self, o):
        return self + (-o)

    def scale(self, c):
        return Sg(self.v * np.float32(c * self.s), 1)

    def val(self):
        return self.v if self.s > 0 else -self.v


def _dft4_finish(t0, t1, t2, t3, sgn):
    X0 = (t0[0] + t2[0], t0[1] + t2[1])
    X2 = (t0[0] - t2[0], t0[1] - t2[1])
    XA = (t1[0] + t3[1], t1[1] - t3[0])
    XB = (t1[0] - t3[1], t1[1] + t3[0])
    if sgn < 0:
        return [X0, XA, X2, XB]
    return [X0, XB, X2, XA]


def _dft4(x, sgn):
    (r0, i0), (r1, i1), (r2, i2), (r3, i3) = x
    return _dft4_finish((r0 + r2, i0 + i2), (r0 - r2, i0 - i2), (r1 + r3, i1 + i3), (r1 - r3, i1 - i3), sgn)


def _dft4_one(x, k, sgn):
    if k % 2 == 0:
        t0 = (x[0][0] + x[2][0], x[0][1] + x[2][1])
        t2 = (x[1][0] + x[3][0], x[1][1] + x[3][1])
        return (t0[0] + t2[0], t0[1] + t2[1]) if k == 0 else (t0[0] - t2[0], t0[1] - t2[1])
    t1 = (x[0][0] - x[2][0], x[0][1] - x[2][1])
    t3 = (x[1][0] - x[3][0], x[1][1] - x[3][1])
    if (k == 1) == (sgn < 0):
        return (t1[0] + t3[1], t1[1] - t3[0])
    return (t1[0] - t3[1], t1[1] + t3[0])


def _dft4_two(x, par, sgn):
    if par == 0:
        t0 = (x[0][0] + x[2][0], x[0][1] + x[2][1])
        t2 = (x[1][0] + x[3][0], x[1][1] + x[3][1])
        return [(t0[0] + t2[0], t0[1] + t2[1]), (t0[0] - t2[0], t0[1] - t2[1])]
    t1 = (x[0][0] - x[2][0], x[0][1] - x[2][1])
    t3 = (x[1][0] - x[3][0], x[1][1] - x[3][1])
    xa = (t1[0] + t3[1], t1[1] - t3[0])
    xb = (t1[0] - t3[1], t1[1] + t3[0])
    return [xa, xb] if sgn < 0 else [xb, xa]


def _tw16(z, e, sgn):
    r, i = z
    e = e % 16
    if e == 0:
        return z
    if e == 4:
        return (i, -r) if sgn < 0 else (-i, r)
    if e == 8:
        return (-r, -i)
    if e == 12:
        return (-i, r) if sgn < 0 else (i, -r)
    h = float(np.sqrt(0.5))
    if e in (2, 6, 10, 14):
        c = h if e in (2, 14) else -h
        s = h * sgn * (1 if e < 8 else -1)
        re = (r if c > 0 else -r) - (i if s > 0 else -i)
        im = (r if s > 0 else -r) + (i if c > 0 else -i)
        return (re.scale(h), im.scale(h))
    c = float(np.cos(2 * np.pi * e / 16))
    s = float(sgn * np.sin(2 * np.pi * e / 16))
    return (r.scale(c) - i.scale(s), r.scale(s) + i.scale(c))


def _sg(z):
    return (Sg(z[0]), Sg(z[1]))


def _bf_lo(u):
    return pltpu.bitcast(u << 16, f32)


def _bf_hi(u):
    return pltpu.bitcast(u & np.uint32(0xFFFF0000), f32)


def _asbf(u):
    return pltpu.bitcast(u, bf16)


import contextlib


def _make_kernel(FC, WWAITS, WSTART, P0MODE, T2AHEAD, XPRI, XG, FPRI, SCOPES, SPLIT0, SPLITL, OPQ, CM, EM, ANN, MG, THR, OPW, NR, HR):
    def sc(name):
        return jax.named_scope(name) if SCOPES else contextlib.nullcontext()

    NCH = F // FC

    def _kernel(x_hbm, wr_hbm, wi_hbm, wg_hbm, wu_hbm, wd_hbm, f_hbm, g_hbm, b_hbm, o_hbm,
                XS, WS, BUF, WP, VF, FP, YB, FS, GS, BS, MS, WG, WU, WD, OS, AT, ACC,
                zi_ref, sem_x, sem_w, sem_t, sem_m, sem_o):
        wgrp = {t: gi for gi, (_, a, b) in enumerate(WWAITS) for t in range(a, b)}
        xgrp = {j: gi for gi, pairs in enumerate(XG) for j in pairs}
        ct = [pltpu.make_async_copy(b_hbm, BS, sem_t.at[0]),
              pltpu.make_async_copy(f_hbm, FS, sem_t.at[1]),
              pltpu.make_async_copy(g_hbm, GS, sem_t.at[2])]
        cx = [pltpu.make_async_copy(x_hbm.at[:, pl.ds(t * 128, 128)], XS.at[t], sem_x.at[xgrp[t % 8]]) for t in range(16)]
        cw = [[pltpu.make_async_copy(w.at[:, pl.ds(t * 128, 128)], WS.at[c, t], sem_w.at[wgrp[t]]) for t in range(16)]
              for c, w in enumerate((wr_hbm, wi_hbm))]
        cm = [[pltpu.make_async_copy(a.at[:, pl.ds(j * FC, FC)], b.at[:, pl.ds(j * FC, FC)], sem_m.at[j])
               for i, (a, b) in enumerate(((wg_hbm, WG), (wu_hbm, WU), (wd_hbm, WD)))] for j in range(NCH)]
        if not MG:
            ct[0].start(priority=0)
        ct[1].start(priority=FPRI)
        for gi, pairs in enumerate(XG):
            for j in pairs:
                cx[j].start(priority=XPRI[gi])
                cx[j + 8].start(priority=XPRI[gi])
        if MG:
            ct[0].start(priority=1)

        if ANN:
            XS, WS, FS, GS, BS, WG, WU, WD = [pltpu.annotate(r, no_store=True) for r in (XS, WS, FS, GS, BS, WG, WU, WD)]
        row8 = jax.lax.broadcasted_iota(jnp.int32, (8, 128), 0)
        rev8 = 7 - row8

        def _zero(i, carry):
            zi_ref[i] = 0
            return carry
        jax.lax.fori_loop(0, 16, _zero, 0)

        def gen_m(d):
            gr, gi_ = BS[0:8, :], BS[8:16, :]
            ur, ui = BS[16:32, :], BS[32:48, :]
            if d == 0:
                c_r, c_i = ur, ui
            else:
                twr = jnp.broadcast_to(BS[48 + d:49 + d, :], (16, 128))
                twi = jnp.broadcast_to(BS[64 + d:65 + d, :], (16, 128))
                c_r = ur * twr - ui * twi
                c_i = ur * twi + ui * twr
            for q2 in range(8):
                m0, m1, m2, m3 = [], [], [], []
                for q in (2 * q2, 2 * q2 + 1):
                    cr = jnp.broadcast_to(c_r[q:q + 1, :], (8, 128))
                    ci = jnp.broadcast_to(c_i[q:q + 1, :], (8, 128))
                    mr = gr * cr - gi_ * ci
                    mi = gr * ci + gi_ * cr
                    m0.append(mr)
                    m1.append(mr + mi)
                    m2.append(mr - mi)
                    m3.append(mi)
                for k_, m in enumerate((m0, m1, m2, m3)):
                    if (k_ in (1, 2) and 3 not in (CM, EM)) or (k_ == 3 and 4 not in (CM, EM)):
                        continue
                    MS[d, k_, pl.ds(16 * q2, 16), :] = jnp.concatenate(m, axis=0).astype(bf16)

        if MG == 0:
            with sc("w_tab"):
                ct[0].wait()
            for d in range(16):
                gen_m(d)
        with sc("w_f"):
            ct[1].wait()

        def fold_tile(t):
            def ld(v, reverse):
                u = pltpu.bitcast(XS[t, pl.ds(16 * v, 16), :], u32)
                if reverse:
                    u = jnp.take_along_axis(u, rev8, axis=0)
                return _bf_lo(u), _bf_hi(u)
            Ree, Ro, Ie, Io = [], [], [], []
            sq = None
            for v in range(7):
                Al, Ah = ld(v, False)
                Bl, Bh = ld(27 - v, True)
                Cl, Ch = ld(13 - v, True)
                Dl, Dh = ld(14 + v, False)
                for (a, b, c, d) in ((Al, Bh, Ch, Dl), (Ah, Bl, Cl, Dh)):
                    p = a + b
                    q = c + d
                    r = a - b
                    s = d - c
                    ro, ie, io = q - p, s + r, s - r
                    Ree.append(q + p)
                    Ro.append(ro)
                    Ie.append(ie)
                    Io.append(io)
                    t2 = ro * ro + ie * ie + io * io
                    sq = t2 if sq is None else sq + t2
            tot = Ree[0]
            for z in Ree[1:]:
                tot = tot + z
            mean4 = jnp.sum(tot, axis=0, keepdims=True) * np.float32(4.0 / D)
            Ree = [z - mean4 for z in Ree]
            for z in Ree:
                sq = sq + z * z
            var = jnp.sum(sq, axis=0, keepdims=True) * np.float32(1.0 / (4 * D))
            rstd = jax.lax.rsqrt(var + EPS)
            return (Ree, Ie, Ro, Io), rstd

        def stage_a(j):
            parts = [fold_tile(j), fold_tile(j + 8)]
            rstd = jnp.concatenate([p[1] for p in parts], axis=1)
            zpad = jnp.zeros((16, 256), f32)
            for odd in (1, 0):
                z = []
                for blk in (2 * odd, 2 * odd + 1):
                    rows = [jnp.concatenate([parts[i][0][blk][v] for i in range(2)], axis=1) for v in range(14)]
                    data = jnp.concatenate(rows + [zpad], axis=0).astype(bf16)
                    nrow = 56 if odd else 64
                    z.append(jnp.dot(_asbf(FS[blk, 0:nrow, :]), data, preferred_element_type=f32))
                for g in range(15 - odd):
                    rs = pl.ds(16 * g + 8 * odd, 8)
                    zr = z[0][8 * g:8 * g + 8, :] * rstd
                    zi = z[1][8 * g:8 * g + 8, :] * rstd
                    xa = (Sg(zr[:, 0:128]), Sg(zi[:, 0:128]))
                    xb = (Sg(zr[:, 128:256]), Sg(zi[:, 128:256]))
                    sm = (xa[0] + xb[0], xa[1] + xb[1])
                    df = _tw16((xa[0] - xb[0], xa[1] - xb[1]), j, -1)
                    VF[0, 0, j, rs, :] = sm[0].val()
                    VF[1, 0, j, rs, :] = sm[1].val()
                    VF[0, 1, j, rs, :] = df[0].val()
                    VF[1, 1, j, rs, :] = df[1].val()

        for gi, pairs in enumerate(XG):
            with sc("w_x"):
                for j in pairs:
                    cx[j].wait()
                    cx[j + 8].wait()
            if gi == WSTART:
                for t in range(16):
                    cw[0][t].start(priority=1)
                    cw[1][t].start(priority=1)
            if gi == len(XG) - 1:
                ct[2].start(priority=1)
                for c in cm[0]:
                    c.start(priority=1)
            for j in pairs:
                stage_a(j)
            if MG and gi == len(XG) - 1:
                with sc("w_tab"):
                    ct[0].wait()
                gen_m(0)
                gen_m(8)

        NWT = 2 * 16 * 8 * WPITCH

        def wt_row(c, t, z=0):
            return (c * 16 + t) * 8 * WPITCH + z

        def vi_rows(c, par, d, gam, z=0):
            r = NWT + ((c * 2 + par) * 8 + d) * 8 * NG + 8 * gam + z
            return pl.ds(r if isinstance(r, int) else pl.multiple_of(r, 8), 8)

        def t1(t, c):
            u = pltpu.bitcast(WS[c, t, 0:224, :], u32)
            w224 = pltpu.bitcast(WS[c, t, 224:225, :].astype(f32), u32) >> 16
            last = jnp.where(row8 == 0, jnp.broadcast_to(w224, (8, 128)), np.uint32(0))
            full = jnp.concatenate([u, last, jnp.zeros((8, 128), u32)], axis=0)
            ut = pltpu.bitcast(full, f32).T
            for q in range(8):
                BUF[pl.ds(wt_row(c, t) + WPITCH * q, 16), :] = ut[16 * q:16 * q + 16, :]

        def t2(d, c):
            z = zi_ref[d % 8] if THR else 0
            Gm = jnp.concatenate([BUF[pl.ds(wt_row(c, t, z) + d, 8, stride=WPITCH), :] for t in range(16)], axis=0)
            WP[c, d] = Gm.T[0:120, :]

        def three_dots(zr, zi, d, nt):
            pad = [jnp.zeros((8, 128), f32)]
            ls = [jnp.concatenate([a_ + b_ for a_, b_ in zip(zr, zi)] + pad, axis=0).astype(bf16),
                  jnp.concatenate(zi + pad, axis=0).astype(bf16),
                  jnp.concatenate(zr + pad, axis=0).astype(bf16)]
            if nt:
                ms = (MS[d, 0], MS[d, 1], MS[d, 2])
                k = [jax.lax.dot_general(l, m, NTDIMS, preferred_element_type=f32) for l, m in zip(ls, ms)]
            else:
                ms = (MS[d, 0], MS[d, 2], MS[d, 1])
                k = [jnp.dot(l, m, preferred_element_type=f32) for l, m in zip(ls, ms)]
            out = []
            for gam in range(NG):
                r = slice(8 * gam, 8 * gam + 8)
                out.append((k[0][r] - k[1][r], k[0][r] - k[2][r]))
            return out

        def four_dots(zr, zi, d, nt):
            rows = []
            for a_, b_ in zip(zr, zi):
                rows += [a_, b_]
            lhs = jnp.concatenate(rows, axis=0).astype(bf16)
            if nt:
                A = jax.lax.dot_general(lhs, MS[d, 0], NTDIMS, preferred_element_type=f32)
                B = jax.lax.dot_general(lhs, MS[d, 3], NTDIMS, preferred_element_type=f32)
            else:
                A = jnp.dot(lhs, MS[d, 0], preferred_element_type=f32)
                B = jnp.dot(lhs, MS[d, 3], preferred_element_type=f32)
            out = []
            for gam in range(NG):
                r = 16 * gam
                if nt:
                    out.append((A[r:r + 8] - B[r + 8:r + 16], B[r:r + 8] + A[r + 8:r + 16]))
                else:
                    out.append((A[r:r + 8] + B[r + 8:r + 16], A[r + 8:r + 16] - B[r:r + 8]))
            return out

        def stage_c(d):
            par, dp = d % 2 + (zi_ref[d] if OPQ else 0), d // 2
            ar, ai, br, bi = [], [], [], []
            for gam in range(NG):
                rs = pl.ds(8 * gam, 8)
                v = [(Sg(VF[0, par, j, rs, :]), Sg(VF[1, par, j, rs, :])) for j in range(8)]
                e4 = _dft4_one([v[0], v[2], v[4], v[6]], dp, -1)
                o4 = _tw16(_dft4_one([v[1], v[3], v[5], v[7]], dp, -1), 2 * dp, -1)
                ar.append((e4[0] + o4[0]).val())
                ai.append((e4[1] + o4[1]).val())
                br.append((e4[0] - o4[0]).val())
                bi.append((e4[1] - o4[1]).val())
            for dd, zr, zi in ((d, ar, ai), (d + 8, br, bi)):
                out = (three_dots if CM == 3 else four_dots)(zr, zi, dd, True)
                for gam in range(NG):
                    FP[0, dd, pl.ds(8 * gam, 8), :] = out[gam][0]
                    FP[1, dd, pl.ds(8 * gam, 8), :] = out[gam][1]

        passes = list(range(8))
        wwait = {p: (a, b) for (p, a, b) in WWAITS}
        pending, per = [], 0
        for p in passes:
            if p in wwait:
                a, b = wwait[p]
                with sc("w_w"):
                    for t in range(a, b):
                        cw[0][t].wait()
                        cw[1][t].wait()
                pending = [(t, c) for t in range(a, b) for c in range(2)]
                nxt = [q for q in sorted(wwait) if q > p]
                span = (nxt[0] if nxt else len(passes)) - p
                per = -(-len(pending) // span)
            for (t, c) in pending[:per]:
                t1(t, c)
            pending = pending[per:]
            if MG and p + 1 < 8:
                gen_m(p + 1)
                gen_m(p + 9)
            stage_c(p)
        assert not pending

        def w_mul(d):
            pr, pi = [], []
            for gam in range(NG):
                gg, odd = gam // 2, gam % 2
                wu_r = pltpu.bitcast(WP[0, d, pl.ds(8 * gg, 8), :], u32)
                wu_i = pltpu.bitcast(WP[1, d, pl.ds(8 * gg, 8), :], u32)
                wr_ = _bf_hi(wu_r) if odd else _bf_lo(wu_r)
                wi_ = _bf_hi(wu_i) if odd else _bf_lo(wu_i)
                zr = FP[0, d, pl.ds(8 * gam, 8), :]
                zi = FP[1, d, pl.ds(8 * gam, 8), :]
                pr.append(zr * wr_ - zi * wi_)
                pi.append(zr * wi_ + zi * wr_)
            return (three_dots if EM == 3 else four_dots)(pr, pi, d, False)

        def stage_e(d):
            ua = w_mul(d)
            ub = w_mul(d + 8)
            for gam in range(NG):
                rs = pl.ds(8 * gam, 8)
                xa, xb = _sg(ua[gam]), _sg(ub[gam])
                sm = (xa[0] + xb[0], xa[1] + xb[1])
                df = _tw16((xa[0] - xb[0], xa[1] - xb[1]), d, +1)
                z = zi_ref[8 + d] if THR else 0
                BUF[vi_rows(0, 0, d, gam, z), :] = sm[0].val()
                BUF[vi_rows(1, 0, d, gam, z), :] = sm[1].val()
                BUF[vi_rows(0, 1, d, gam, z), :] = df[0].val()
                BUF[vi_rows(1, 1, d, gam, z), :] = df[1].val()

        t2jobs = [[(d + 8 * s_, c) for s_ in range(2) for c in range(2)] for d in range(8)]
        for p in range(T2AHEAD):
            for (d, c) in t2jobs[p]:
                t2(d, c)
        for p in range(8):
            if not THR and p + T2AHEAD < 8:
                for (d, c) in t2jobs[p + T2AHEAD]:
                    t2(d, c)
            stage_e(p)
            if THR and p + T2AHEAD < 8:
                for (d, c) in t2jobs[p + T2AHEAD]:
                    t2(d, c)

        with sc("w_g"):
            ct[2].wait()

        def revrows(z):
            nq = z.shape[0] // 8
            idx = 7 - jax.lax.broadcasted_iota(jnp.int32, (8, z.shape[1]), 0)
            return jnp.concatenate(
                [jnp.take_along_axis(z[8 * q:8 * q + 8], idx, axis=0) for q in range(nq - 1, -1, -1)], axis=0)

        def prep_a(i):
            par, typ = i % 2, i // 2
            zz = zi_ref[8 + i] if OPQ else 0
            Y = []
            for gam in range(NG):
                rs = pl.ds(8 * gam, 8)
                w = [(Sg(BUF[vi_rows(0, par, d, gam, zz), :]), Sg(BUF[vi_rows(1, par, d, gam, zz), :])) for d in range(8)]
                ev = _dft4_two([w[0], w[2], w[4], w[6]], typ, +1)
                od = _dft4_two([w[1], w[3], w[5], w[7]], typ, +1)
                outs = {}
                for kk, bp in enumerate((typ, typ + 2)):
                    o4 = _tw16(od[kk], 2 * bp, +1)
                    outs[bp] = (ev[kk][0] + o4[0], ev[kk][1] + o4[1])
                    outs[bp + 4] = (ev[kk][0] - o4[0], ev[kk][1] - o4[1])
                X = [outs[typ + 2 * b1] for b1 in range(4)]
                Y.append((jnp.concatenate([X[b1][0].val() for b1 in range(4)], axis=1),
                          jnp.concatenate([X[b1][1].val() for b1 in range(4)], axis=1)))
            zero = jnp.zeros((8, BM), f32)
            for blk in range(4):
                c, odd = blk % 2, blk // 2
                ng = 15 - odd
                for q in range(8):
                    rows = [Y[2 * g + odd][c] if g < ng else zero for g in (2 * q, 2 * q + 1)]
                    YB[i % 2, blk, pl.ds(16 * q, 16), :] = jnp.concatenate(rows, axis=0).astype(bf16)

        def prep_d(i, l0=0, l1=4):
            ls = slice(128 * l0, 128 * l1)
            Ce = jnp.dot(_asbf(GS[0]), YB[i % 2, 0, :, ls], preferred_element_type=f32)
            Se = jnp.dot(_asbf(GS[1]), YB[i % 2, 1, :, ls], preferred_element_type=f32)
            Co = jnp.dot(_asbf(GS[2]), YB[i % 2, 2, :, ls], preferred_element_type=f32)
            So = jnp.dot(_asbf(GS[3]), YB[i % 2, 3, :, ls], preferred_element_type=f32)
            return Ce, Se, Co, So

        def prep_b(i, z, l0=0, l1=4):
            Ce, Se, Co, So = z
            ls = slice(128 * l0, 128 * l1)
            pp = Ce + Co
            mm = Ce - Co
            qq = Se + So
            rr = So - Se
            y = jnp.concatenate([mm + rr, revrows(pp + qq), pp - qq, revrows(mm - rr)], axis=0)
            xw = jnp.concatenate([XS[i + 4 * b1] for b1 in range(l0, l1)], axis=1)
            h = xw.astype(f32) + y
            if HR:
                h = h.astype(bf16).astype(f32)
            mu = jnp.mean(h, axis=0, keepdims=True)
            hc = h - mu
            var = jnp.mean(hc * hc, axis=0, keepdims=True)
            a = (hc * jax.lax.rsqrt(var + EPS)).astype(bf16)
            AT[i, ls, :] = a.T
            ACC[i, :, ls] = h

        def fslice(i, j):
            if OPW and isinstance(i, int):
                return pl.ds(pl.multiple_of(j * FC + zi_ref[12 + i], 128), FC)
            return slice(j * FC, (j + 1) * FC)

        def mlp_up(i, j, l0=0, l1=4):
            sl = fslice(i, j)
            at = AT[i, 128 * l0:128 * l1, :]
            g = jnp.dot(at, WG[:, sl], preferred_element_type=f32)
            u = jnp.dot(at, WU[:, sl], preferred_element_type=f32)
            return (g * u).astype(bf16)

        def mlp_down(i, j, hh, l0=0, l1=4):
            sl = fslice(i, j)
            ls = slice(128 * l0, 128 * l1)
            if j == NCH - 1:
                nr = D // NR
                for rp in range(NR):
                    rs = slice(rp * nr, (rp + 1) * nr)
                    acc = ACC[i, rs, ls] + jax.lax.dot_general(WD[rs, sl], hh, NTDIMS, preferred_element_type=f32)
                    ob = acc.astype(bf16)
                    for b1 in range(l0, l1):
                        OS[i + 4 * b1, rs, :] = ob[:, 128 * (b1 - l0):128 * (b1 - l0) + 128]
                    for b1 in range(l0, l1):
                        out_copy(i + 4 * b1, rp).start()
            else:
                ACC[i, :, ls] = ACC[i, :, ls] + jax.lax.dot_general(WD[:, sl], hh, NTDIMS, preferred_element_type=f32)

        def do_mlp(i, j, l0=0, l1=4):
            mlp_down(i, j, mlp_up(i, j, l0, l1), l0, l1)

        def out_copy(t, rp):
            off = t * 128 if isinstance(t, int) else pl.multiple_of(t * 128, 128)
            nr = D // NR
            return pltpu.make_async_copy(OS.at[t, pl.ds(rp * nr, nr), :],
                                         o_hbm.at[pl.ds(rp * nr, nr), pl.ds(off, 128)], sem_o.at[0])

        prep_a(0)
        if SPLIT0:
            prep_b(0, prep_d(0, 0, 2), 0, 2)
        else:
            prep_b(0, prep_d(0))
        for j in range(NCH):
            with sc("w_m"):
                for c in cm[j]:
                    c.wait()
            if j + 1 < NCH:
                for c in cm[j + 1]:
                    c.start()
            if j == 0:
                for i in range(NB):
                    if i == 0 and SPLIT0:
                        z = prep_d(0, 2, 4)
                        hh = mlp_up(0, 0, 0, 2)
                        prep_b(0, z, 2, 4)
                        mlp_down(0, 0, hh, 0, 2)
                        prep_a(1)
                        hh = mlp_up(0, 0, 2, 4)
                        z = prep_d(1)
                        mlp_down(0, 0, hh, 2, 4)
                        prep_b(1, z)
                        continue
                    if i + 1 < NB:
                        prep_a(i + 1)
                    hh = mlp_up(i, 0)
                    if i + 1 < NB:
                        z = prep_d(i + 1)
                    mlp_down(i, 0, hh)
                    if i + 1 < NB:
                        prep_b(i + 1, z)
            elif P0MODE == "unroll":
                for i in range(NB):
                    do_mlp(i, j)
            else:
                nloop = NB - 1 if (SPLITL and j == NCH - 1) else NB

                def body(i, carry, j=j):
                    do_mlp(i, j)
                    return carry
                jax.lax.fori_loop(0, nloop, body, 0)
                if nloop < NB:
                    for (l0, l1) in SPLITL:
                        do_mlp(NB - 1, j, l0, l1)
        with sc("w_out"):
            for t in range(16):
                for rp in range(NR):
                    out_copy(t, rp).wait()
    return _kernel


def build(interpret=False, FC=896, WWAITS=((2, 0, 8), (6, 8, 16)), WSTART=1, P0MODE="loop", T2AHEAD=1, XPRI=(1, 1, 1, 1), XG=((0, 1), (2, 3), (4, 5), (6, 7)), FPRI=0, SCOPES=False, SPLIT0=True, SPLITL=(), OPQ=True, CM=3, EM=3, ANN=False, MG=0, THR=False, OPW=False, NR=4, HR=False, fl=()):
    names = dict(lp='XLA_TPU_FORCE_LP_LLO_SCHEDULER', ev='XLA_TPU_EVENLY_DISTRIBUTE_CRITICAL_NODES', dd='XLA_TPU_RESCHEDULE_DMA_DONES', sl='XLA_TPU_ENABLE_LLO_SMALL_LOOP_FLATTENING')
    flags = {names[k]: True for k in fl} or None

    def fn(A_x, A_w_r, A_w_i, B_x, B_w_gate, B_w_up, B_w_down):
        Ft, G, base = _tables()
        xt = jnp.transpose(A_x, (0, 2, 1)).reshape(D, S)
        any_spec = pl.BlockSpec(memory_space=pl.ANY)
        R = 8 * NG
        out = pl.pallas_call(
            _make_kernel(FC, WWAITS, WSTART, P0MODE, T2AHEAD, XPRI, XG, FPRI, SCOPES, SPLIT0, SPLITL, OPQ, CM, EM, ANN, MG, THR, OPW, NR, HR),
            out_shape=jax.ShapeDtypeStruct((D, S), bf16),
            in_specs=[any_spec] * 9,
            out_specs=any_spec,
            scratch_shapes=[
                pltpu.VMEM((16, D, 128), bf16),
                pltpu.VMEM((2, 16, K, 128), bf16),
                pltpu.VMEM((2 * 16 * 8 * WPITCH + 32 * R, 128), f32),
                pltpu.VMEM((2, 16, 120, 128), f32),
                pltpu.VMEM((2, 2, 8, R, 128), f32),
                pltpu.VMEM((2, 16, R, 128), f32),
                pltpu.VMEM((2, 4, 128, BM), bf16),
                pltpu.VMEM((4, 64, 128), u32),
                pltpu.VMEM((4, 56, 128), u32),
                pltpu.VMEM((80, 128), f32),
                pltpu.VMEM((16, 4, 128, 128), bf16),
                pltpu.VMEM((D, F), bf16),
                pltpu.VMEM((D, F), bf16),
                pltpu.VMEM((D, F), bf16),
                pltpu.VMEM((16, D, 128), bf16),
                pltpu.VMEM((NB, BM, D), bf16),
                pltpu.VMEM((NB, D, BM), f32),
                pltpu.SMEM((16,), jnp.int32),
                pltpu.SemaphoreType.DMA((len(XG),)),
                pltpu.SemaphoreType.DMA((len(WWAITS),)),
                pltpu.SemaphoreType.DMA((3,)),
                pltpu.SemaphoreType.DMA((F // FC,)),
                pltpu.SemaphoreType.DMA((1,)),
            ],
            compiler_params=pltpu.CompilerParams(vmem_limit_bytes=100 * 2**20, flags=flags),
            interpret=(pltpu.InterpretParams() if interpret else False),
        )(xt, A_w_r.T, A_w_i.T, B_w_gate, B_w_up, B_w_down.T, jnp.asarray(Ft), jnp.asarray(G), jnp.asarray(base))
        return jnp.transpose(out.reshape(1, D, S), (0, 2, 1))
    return jax.jit(fn)


_forward = build()


@jax.jit
def pallas_sequential_preLN__spectral_gfnet__glu_gated_bilinear__prompt_kernel(
    A_x: jax.Array,
    A_w_r: jax.Array,
    A_w_i: jax.Array,
    B_x: jax.Array,
    B_w_gate: jax.Array,
    B_w_up: jax.Array,
    B_w_down: jax.Array,
):
    return _forward(A_x, A_w_r, A_w_i, B_x, B_w_gate, B_w_up, B_w_down)
```

```python
import numpy as np
import jax
import jax.numpy as jnp
import jax.experimental.pallas as pl
import jax.experimental.pallas.tpu as pltpu

S, D, F, K = 2048, 448, 1792, 225
EPS = 1e-5
bf16, f32, u32 = jnp.bfloat16, jnp.float32, jnp.uint32
NTDIMS = (((1,), (1,)), ((), ()))
NG = 29
WPITCH = 17
NB = 4
BM = S // NB
FCS = (384, 1408)
FOFF = (0, 384)
NR = 4
WWAITS = {2: (0, 8), 6: (8, 16)}


def _pack_rows(a):
    import ml_dtypes
    b = a.astype(ml_dtypes.bfloat16).view(np.uint16).astype(np.uint32)
    return b[..., 0::2, :] | (b[..., 1::2, :] << 16)


def _tables():
    th = 2 * np.pi / D
    kE = 2 * np.arange(113)
    kO = 2 * np.arange(112) + 1
    n = []
    for v in range(7):
        n += [16 * v + 2 * i for i in range(8)] + [16 * v + 2 * i + 1 for i in range(8)]
    nuf = np.array(n) + 0.5
    Ft = np.zeros((4, 128, 128))
    Ft[0, :112, :112] = np.cos(np.outer(kE[:112], nuf) * th)
    Ft[1, 1:113, :112] = -np.sin(np.outer(kE[1:], nuf) * th)
    Ft[2, :112, :112] = np.cos(np.outer(kO, nuf) * th)
    Ft[3, :112, :112] = -np.sin(np.outer(kO, nuf) * th)
    nu = np.arange(112) + 0.5
    cE = np.full(113, 2.0)
    cE[0] = cE[112] = 1.0
    sc = 1.0 / (D * S)
    G = np.zeros((4, 112, 128))
    G[0, :, :112] = (np.cos(np.outer(nu, kE) * th) * cE * sc)[:, :112]
    G[1, :, 1:113] = (np.sin(np.outer(nu, kE) * th) * cE * sc)[:, 1:]
    G[2, :, :112] = np.cos(np.outer(nu, kO) * th) * 2 * sc
    G[3, :, :112] = np.sin(np.outer(nu, kO) * th) * 2 * sc
    a = np.arange(128)
    pg = -2 * np.pi * (np.outer(np.arange(8), a) % 128) / 128
    pu = -2 * np.pi * (np.outer(8 * np.arange(16), a) % 128) / 128
    pt = -2 * np.pi * np.outer(np.arange(16), a) / S
    seeds = np.concatenate([np.cos(pg), np.sin(pg), np.cos(pu), np.sin(pu), np.cos(pt), np.sin(pt)]).astype(np.float32)
    return _pack_rows(Ft), _pack_rows(G), seeds


class _Sg:
    __slots__ = ("v", "s")

    def __init__(self, v, s=1):
        self.v, self.s = v, s

    def __neg__(self):
        return _Sg(self.v, -self.s)

    def __add__(self, o):
        if self.s == o.s:
            return _Sg(self.v + o.v, self.s)
        if self.s > 0:
            return _Sg(self.v - o.v, 1)
        return _Sg(o.v - self.v, 1)

    def __sub__(self, o):
        return self + (-o)

    def scale(self, c):
        return _Sg(self.v * np.float32(c * self.s), 1)

    def val(self):
        return self.v if self.s > 0 else -self.v


def _cadd(a, b):
    return (a[0] + b[0], a[1] + b[1])


def _csub(a, b):
    return (a[0] - b[0], a[1] - b[1])


def _dft4_pair(x, par, sgn):
    if par == 0:
        t0, t2 = _cadd(x[0], x[2]), _cadd(x[1], x[3])
        return [_cadd(t0, t2), _csub(t0, t2)]
    t1, t3 = _csub(x[0], x[2]), _csub(x[1], x[3])
    xa = (t1[0] + t3[1], t1[1] - t3[0])
    xb = (t1[0] - t3[1], t1[1] + t3[0])
    return [xa, xb] if sgn < 0 else [xb, xa]


def _dft4_one(x, k, sgn):
    if k % 2 == 0:
        t0, t2 = _cadd(x[0], x[2]), _cadd(x[1], x[3])
        return _cadd(t0, t2) if k == 0 else _csub(t0, t2)
    t1, t3 = _csub(x[0], x[2]), _csub(x[1], x[3])
    if (k == 1) == (sgn < 0):
        return (t1[0] + t3[1], t1[1] - t3[0])
    return (t1[0] - t3[1], t1[1] + t3[0])


def _tw16(z, e, sgn):
    r, i = z
    if e == 0:
        return z
    if e == 4:
        return (i, -r) if sgn < 0 else (-i, r)
    if e in (2, 6):
        h = float(np.sqrt(0.5))
        c, s = (1 if e == 2 else -1), sgn
        re = (r if c > 0 else -r) - (i if s > 0 else -i)
        im = (r if s > 0 else -r) + (i if c > 0 else -i)
        return (re.scale(h), im.scale(h))
    c = float(np.cos(2 * np.pi * e / 16))
    s = float(sgn * np.sin(2 * np.pi * e / 16))
    return (r.scale(c) - i.scale(s), r.scale(s) + i.scale(c))


def _bf_lo(u):
    return pltpu.bitcast(u << 16, f32)


def _bf_hi(u):
    return pltpu.bitcast(u & np.uint32(0xFFFF0000), f32)


def _asbf(u):
    return pltpu.bitcast(u, bf16)


def _kernel(x_hbm, wr_hbm, wi_hbm, wg_hbm, wu_hbm, wd_hbm, f_hbm, g_hbm, b_hbm, o_hbm,
            XS, WS, WT, WP, VF, FP, VI, YB, FS, GS, BS, MS, WG, WU, WD, OS, AT, ACC,
            zi, sem_x, sem_w, sem_t, sem_m, sem_o):
    c_seed = pltpu.make_async_copy(b_hbm, BS, sem_t.at[0])
    c_f = pltpu.make_async_copy(f_hbm, FS, sem_t.at[1])
    c_g = pltpu.make_async_copy(g_hbm, GS, sem_t.at[2])
    cx = [pltpu.make_async_copy(x_hbm.at[:, pl.ds(t * 128, 128)], XS.at[t], sem_x.at[(t % 8) // 2])
          for t in range(16)]
    cw = [[pltpu.make_async_copy(w.at[:, pl.ds(t * 128, 128)], WS.at[c, t], sem_w.at[t // 8]) for t in range(16)]
          for c, w in enumerate((wr_hbm, wi_hbm))]
    cm = [[pltpu.make_async_copy(a.at[:, pl.ds(FOFF[j], FCS[j])], b.at[:, pl.ds(FOFF[j], FCS[j])], sem_m.at[j])
           for a, b in ((wg_hbm, WG), (wu_hbm, WU), (wd_hbm, WD))] for j in range(2)]

    def out_copy(t, rp):
        off = t * 128 if isinstance(t, int) else pl.multiple_of(t * 128, 128)
        rows = pl.ds(rp * (D // NR), D // NR)
        return pltpu.make_async_copy(OS.at[t, rows, :], o_hbm.at[rows, pl.ds(off, 128)], sem_o.at[0])

    c_seed.start(priority=0)
    c_f.start(priority=0)
    for j in range(8):
        cx[j].start(priority=1)
        cx[j + 8].start(priority=1)

    def _zero(i, carry):
        zi[i] = 0
        return carry
    jax.lax.fori_loop(0, 16, _zero, 0)

    row8 = jax.lax.broadcasted_iota(jnp.int32, (8, 128), 0)
    rev8 = 7 - row8

    c_seed.wait()
    for d in range(16):
        gr, gi = BS[0:8, :], BS[8:16, :]
        c_r, c_i = BS[16:32, :], BS[32:48, :]
        if d:
            twr = jnp.broadcast_to(BS[48 + d:49 + d, :], (16, 128))
            twi = jnp.broadcast_to(BS[64 + d:65 + d, :], (16, 128))
            c_r, c_i = c_r * twr - c_i * twi, c_r * twi + c_i * twr
        for q2 in range(8):
            ms = ([], [], [])
            for q in (2 * q2, 2 * q2 + 1):
                cr = jnp.broadcast_to(c_r[q:q + 1, :], (8, 128))
                ci = jnp.broadcast_to(c_i[q:q + 1, :], (8, 128))
                mr = gr * cr - gi * ci
                mi = gr * ci + gi * cr
                ms[0].append(mr)
                ms[1].append(mr + mi)
                ms[2].append(mr - mi)
            for k in range(3):
                MS[d, k, pl.ds(16 * q2, 16), :] = jnp.concatenate(ms[k], axis=0).astype(bf16)
    c_f.wait()

    def fold_tile(t):
        def ld(v, reverse):
            u = pltpu.bitcast(XS[t, pl.ds(16 * v, 16), :], u32)
            if reverse:
                u = jnp.take_along_axis(u, rev8, axis=0)
            return _bf_lo(u), _bf_hi(u)
        Ree, Ro, Ie, Io = [], [], [], []
        sq = None
        for v in range(7):
            Al, Ah = ld(v, False)
            Bl, Bh = ld(27 - v, True)
            Cl, Ch = ld(13 - v, True)
            Dl, Dh = ld(14 + v, False)
            for (a, b, c, d) in ((Al, Bh, Ch, Dl), (Ah, Bl, Cl, Dh)):
                p, q, r, s = a + b, c + d, a - b, d - c
                ro, ie, io = q - p, s + r, s - r
                Ree.append(q + p)
                Ro.append(ro)
                Ie.append(ie)
                Io.append(io)
                t2 = ro * ro + ie * ie + io * io
                sq = t2 if sq is None else sq + t2
        tot = Ree[0]
        for z in Ree[1:]:
            tot = tot + z
        mean4 = jnp.sum(tot, axis=0, keepdims=True) * np.float32(4.0 / D)
        Ree = [z - mean4 for z in Ree]
        for z in Ree:
            sq = sq + z * z
        var = jnp.sum(sq, axis=0, keepdims=True) * np.float32(1.0 / (4 * D))
        return (Ree, Ie, Ro, Io), jax.lax.rsqrt(var + EPS)

    def stage_a(j):
        parts = [fold_tile(j), fold_tile(j + 8)]
        rstd = jnp.concatenate([p[1] for p in parts], axis=1)
        zpad = jnp.zeros((16, 256), f32)
        for odd in (1, 0):
            z = []
            for blk in (2 * odd, 2 * odd + 1):
                rows = [jnp.concatenate([parts[i][0][blk][v] for i in range(2)], axis=1) for v in range(14)]
                data = jnp.concatenate(rows + [zpad], axis=0).astype(bf16)
                z.append(jnp.dot(_asbf(FS[blk, 0:(56 if odd else 64), :]), data, preferred_element_type=f32))
            for g in range(15 - odd):
                rs = pl.ds(16 * g + 8 * odd, 8)
                zr = z[0][8 * g:8 * g + 8, :] * rstd
                zm = z[1][8 * g:8 * g + 8, :] * rstd
                xa = (_Sg(zr[:, 0:128]), _Sg(zm[:, 0:128]))
                xb = (_Sg(zr[:, 128:256]), _Sg(zm[:, 128:256]))
                sm = _cadd(xa, xb)
                df = _tw16(_csub(xa, xb), j, -1)
                VF[0, 0, j, rs, :] = sm[0].val()
                VF[1, 0, j, rs, :] = sm[1].val()
                VF[0, 1, j, rs, :] = df[0].val()
                VF[1, 1, j, rs, :] = df[1].val()

    for gi in range(4):
        for j in (2 * gi, 2 * gi + 1):
            cx[j].wait()
            cx[j + 8].wait()
        if gi == 1:
            for t in range(16):
                cw[0][t].start(priority=1)
                cw[1][t].start(priority=1)
        stage_a(2 * gi)
        stage_a(2 * gi + 1)

    def t1(t, c):
        u = pltpu.bitcast(WS[c, t, 0:224, :], u32)
        w224 = pltpu.bitcast(WS[c, t, 224:225, :].astype(f32), u32) >> 16
        last = jnp.where(row8 == 0, jnp.broadcast_to(w224, (8, 128)), np.uint32(0))
        full = jnp.concatenate([u, last, jnp.zeros((8, 128), u32)], axis=0)
        ut = pltpu.bitcast(full, f32).T
        for q in range(8):
            WT[c, t, pl.ds(WPITCH * q, 16), :] = ut[16 * q:16 * q + 16, :]

    def t2(d, c):
        gm = jnp.concatenate([WT[c, t, pl.ds(d, 8, stride=WPITCH), :] for t in range(16)], axis=0)
        WP[c, d] = gm.T[0:120, :]

    def three_dots(zr, zm, d, forward):
        pad = [jnp.zeros((8, 128), f32)]
        ls = [jnp.concatenate([a + b for a, b in zip(zr, zm)] + pad, axis=0).astype(bf16),
              jnp.concatenate(zm + pad, axis=0).astype(bf16),
              jnp.concatenate(zr + pad, axis=0).astype(bf16)]
        if forward:
            k = [jax.lax.dot_general(l, MS[d, m], NTDIMS, preferred_element_type=f32) for l, m in zip(ls, (0, 1, 2))]
        else:
            k = [jnp.dot(l, MS[d, m], preferred_element_type=f32) for l, m in zip(ls, (0, 2, 1))]
        return [(k[0][8 * g:8 * g + 8] - k[1][8 * g:8 * g + 8], k[0][8 * g:8 * g + 8] - k[2][8 * g:8 * g + 8])
                for g in range(NG)]

    def stage_c(d):
        par, dp = d % 2 + zi[d], d // 2
        ar, ai, br, bi = [], [], [], []
        for g in range(NG):
            rs = pl.ds(8 * g, 8)
            v = [(_Sg(VF[0, par, j, rs, :]), _Sg(VF[1, par, j, rs, :])) for j in range(8)]
            e4 = _dft4_one(v[0::2], dp, -1)
            o4 = _tw16(_dft4_one(v[1::2], dp, -1), 2 * dp, -1)
            xa, xb = _cadd(e4, o4), _csub(e4, o4)
            ar.append(xa[0].val())
            ai.append(xa[1].val())
            br.append(xb[0].val())
            bi.append(xb[1].val())
        for dd, zr, zm in ((d, ar, ai), (d + 8, br, bi)):
            out = three_dots(zr, zm, dd, True)
            for g in range(NG):
                FP[0, dd, pl.ds(8 * g, 8), :] = out[g][0]
                FP[1, dd, pl.ds(8 * g, 8), :] = out[g][1]

    pending, per = [], 0
    for p in range(8):
        if p in WWAITS:
            a, b = WWAITS[p]
            for t in range(a, b):
                cw[0][t].wait()
                cw[1][t].wait()
            if b == 16:
                c_g.start(priority=1)
                for c in cm[0]:
                    c.start(priority=1)
            pending = [(t, c) for t in range(a, b) for c in range(2)]
            per = -(-len(pending) // (min([q for q in WWAITS if q > p] + [8]) - p))
        for (t, c) in pending[:per]:
            t1(t, c)
        pending = pending[per:]
        stage_c(p)

    def filtered(d):
        pr, pi = [], []
        for g in range(NG):
            unpack = _bf_hi if g % 2 else _bf_lo
            w_r = unpack(pltpu.bitcast(WP[0, d, pl.ds(8 * (g // 2), 8), :], u32))
            w_i = unpack(pltpu.bitcast(WP[1, d, pl.ds(8 * (g // 2), 8), :], u32))
            zr = FP[0, d, pl.ds(8 * g, 8), :]
            zm = FP[1, d, pl.ds(8 * g, 8), :]
            pr.append(zr * w_r - zm * w_i)
            pi.append(zr * w_i + zm * w_r)
        return three_dots(pr, pi, d, False)

    for d in (0, 8):
        t2(d, 0)
        t2(d, 1)
    for d in range(8):
        if d + 1 < 8:
            for dd in (d + 1, d + 9):
                t2(dd, 0)
                t2(dd, 1)
        ua, ub = filtered(d), filtered(d + 8)
        for g in range(NG):
            rs = pl.ds(8 * g, 8)
            xa, xb = (_Sg(ua[g][0]), _Sg(ua[g][1])), (_Sg(ub[g][0]), _Sg(ub[g][1]))
            sm = _cadd(xa, xb)
            df = _tw16(_csub(xa, xb), d, +1)
            VI[0, 0, d, rs, :] = sm[0].val()
            VI[1, 0, d, rs, :] = sm[1].val()
            VI[0, 1, d, rs, :] = df[0].val()
            VI[1, 1, d, rs, :] = df[1].val()

    def prep_a(i):
        par, typ = i % 2 + zi[8 + i], i // 2
        Y = []
        for g in range(NG):
            rs = pl.ds(8 * g, 8)
            w = [(_Sg(VI[0, par, d, rs, :]), _Sg(VI[1, par, d, rs, :])) for d in range(8)]
            ev = _dft4_pair(w[0::2], typ, +1)
            od = _dft4_pair(w[1::2], typ, +1)
            outs = {}
            for kk, bp in enumerate((typ, typ + 2)):
                o4 = _tw16(od[kk], 2 * bp, +1)
                outs[bp] = _cadd(ev[kk], o4)
                outs[bp + 4] = _csub(ev[kk], o4)
            X = [outs[typ + 2 * b1] for b1 in range(4)]
            Y.append([jnp.concatenate([X[b1][c].val() for b1 in range(4)], axis=1) for c in range(2)])
        zero = jnp.zeros((8, BM), f32)
        for blk in range(4):
            c, odd = blk % 2, blk // 2
            for q in range(8):
                rows = [Y[2 * g + odd][c] if g < 15 - odd else zero for g in (2 * q, 2 * q + 1)]
                YB[i % 2, blk, pl.ds(16 * q, 16), :] = jnp.concatenate(rows, axis=0).astype(bf16)

    def revrows(z):
        idx = 7 - jax.lax.broadcasted_iota(jnp.int32, (8, z.shape[1]), 0)
        return jnp.concatenate([jnp.take_along_axis(z[8 * q:8 * q + 8], idx, axis=0)
                                for q in range(z.shape[0] // 8 - 1, -1, -1)], axis=0)

    def prep_b(i, l0, l1):
        ls = slice(128 * l0, 128 * l1)
        Ce, Se, Co, So = [jnp.dot(_asbf(GS[blk]), YB[i % 2, blk, :, ls], preferred_element_type=f32)
                          for blk in range(4)]
        pp, mm, qq, rr = Ce + Co, Ce - Co, Se + So, So - Se
        y = jnp.concatenate([mm + rr, revrows(pp + qq), pp - qq, revrows(mm - rr)], axis=0)
        h = jnp.concatenate([XS[i + 4 * b1] for b1 in range(l0, l1)], axis=1).astype(f32) + y
        hc = h - jnp.mean(h, axis=0, keepdims=True)
        var = jnp.mean(hc * hc, axis=0, keepdims=True)
        AT[i, ls, :] = (hc * jax.lax.rsqrt(var + EPS)).astype(bf16).T
        ACC[i, :, ls] = h

    def mlp_up(i, j, mid=None):
        sl = slice(FOFF[j], FOFF[j] + FCS[j])
        at = AT[i]
        g = jnp.dot(at, WG[:, sl], preferred_element_type=f32)
        if mid is not None:
            mid()
        u = jnp.dot(at, WU[:, sl], preferred_element_type=f32)
        return (g * u).astype(bf16)

    c_g.wait()
    prep_a(0)
    for l0 in range(4):
        prep_b(0, l0, l0 + 1)
    for c in cm[0]:
        c.wait()
    for c in cm[1]:
        c.start()
    for i in range(NB):
        if i + 1 < NB:
            prep_a(i + 1)
        hh = mlp_up(i, 0, mid=(lambda: prep_b(i + 1, 0, 4)) if i + 1 < NB else None)
        ACC[i] = ACC[i] + jax.lax.dot_general(WD[:, 0:FCS[0]], hh, NTDIMS, preferred_element_type=f32)

    for c in cm[1]:
        c.wait()

    def last_pass(i, carry):
        hh = mlp_up(i, 1)
        for rp in range(NR):
            rs = slice(rp * (D // NR), (rp + 1) * (D // NR))
            ob = (ACC[i, rs, :] + jax.lax.dot_general(WD[rs, FOFF[1]:F], hh, NTDIMS,
                                                      preferred_element_type=f32)).astype(bf16)
            for b1 in range(4):
                OS[i + 4 * b1, rs, :] = ob[:, 128 * b1:128 * b1 + 128]
            for b1 in range(4):
                out_copy(i + 4 * b1, rp).start()
        return carry
    jax.lax.fori_loop(0, NB, last_pass, 0)
    for t in range(16):
        for rp in range(NR):
            out_copy(t, rp).wait()


def _forward(A_x, A_w_r, A_w_i, B_w_gate, B_w_up, B_w_down, interpret=False):
    Ft, G, seeds = _tables()
    any_spec = pl.BlockSpec(memory_space=pl.ANY)
    R = 8 * NG
    out = pl.pallas_call(
        _kernel,
        out_shape=jax.ShapeDtypeStruct((D, S), bf16),
        in_specs=[any_spec] * 9,
        out_specs=any_spec,
        scratch_shapes=[
            pltpu.VMEM((16, D, 128), bf16),
            pltpu.VMEM((2, 16, K, 128), bf16),
            pltpu.VMEM((2, 16, 8 * WPITCH, 128), f32),
            pltpu.VMEM((2, 16, 120, 128), f32),
            pltpu.VMEM((2, 2, 8, R, 128), f32),
            pltpu.VMEM((2, 16, R, 128), f32),
            pltpu.VMEM((2, 2, 8, R, 128), f32),
            pltpu.VMEM((2, 4, 128, BM), bf16),
            pltpu.VMEM((4, 64, 128), u32),
            pltpu.VMEM((4, 56, 128), u32),
            pltpu.VMEM((80, 128), f32),
            pltpu.VMEM((16, 3, 128, 128), bf16),
            pltpu.VMEM((D, F), bf16),
            pltpu.VMEM((D, F), bf16),
            pltpu.VMEM((D, F), bf16),
            pltpu.VMEM((16, D, 128), bf16),
            pltpu.VMEM((NB, BM, D), bf16),
            pltpu.VMEM((NB, D, BM), f32),
            pltpu.SMEM((16,), jnp.int32),
            pltpu.SemaphoreType.DMA((4,)),
            pltpu.SemaphoreType.DMA((2,)),
            pltpu.SemaphoreType.DMA((3,)),
            pltpu.SemaphoreType.DMA((2,)),
            pltpu.SemaphoreType.DMA((1,)),
        ],
        compiler_params=pltpu.CompilerParams(
            vmem_limit_bytes=100 * 2**20,
            flags={"XLA_TPU_EVENLY_DISTRIBUTE_CRITICAL_NODES": True}),
        interpret=interpret,
    )(jnp.transpose(A_x, (0, 2, 1)).reshape(D, S), A_w_r.T, A_w_i.T, B_w_gate, B_w_up, B_w_down.T,
      jnp.asarray(Ft), jnp.asarray(G), jnp.asarray(seeds))
    return jnp.transpose(out.reshape(1, D, S), (0, 2, 1))


@jax.jit
def pallas_sequential_preLN__spectral_gfnet__glu_gated_bilinear__prompt_kernel(
    A_x: jax.Array,
    A_w_r: jax.Array,
    A_w_i: jax.Array,
    B_x: jax.Array,
    B_w_gate: jax.Array,
    B_w_up: jax.Array,
    B_w_down: jax.Array,
):
    del B_x
    return _forward(A_x, A_w_r, A_w_i, B_w_gate, B_w_up, B_w_down)
```
